```python
import os as _os
_os.environ.setdefault('JAX_PLATFORMS', 'cpu')
import jax
import jax.numpy as jnp

def _softmax(x, axis=-1):
    return jax.nn.softmax(x, axis=axis)

def _gelu(x):
    return jax.nn.gelu(x, approximate=True)

def _silu(x):
    return jax.nn.silu(x)

def _sigmoid(x):
    return jax.nn.sigmoid(x)

def _layernorm(x, axis=-1, eps=1e-05):
    m = jnp.mean(x, axis=axis, keepdims=True)
    v = jnp.var(x, axis=axis, keepdims=True)
    return (x - m) / jnp.sqrt(v + eps)

def _scatter_add(tgt, idx, src, axis=0):
    return tgt.at[idx].add(src)

def _segment_sum(src, seg, n):
    return jax.ops.segment_sum(src, seg, n)

class _Rng:

    def __init__(self, key):
        self._k = key

    def _next(self):
        self._k, sub = jax.random.split(self._k)
        return sub

    def normal(self, shape):
        return jax.random.normal(self._next(), shape, dtype=jnp.bfloat16)

    def randint(self, lo, hi, shape):
        return jax.random.randint(self._next(), shape, lo, hi, dtype=jnp.int32)

    def uniform(self, shape, lo=0.0, hi=1.0):
        return jax.random.uniform(self._next(), shape, jnp.bfloat16, lo, hi)

    def permutation(self, n):
        return jax.random.permutation(self._next(), n)
kernel_name = 'adaLN_cond__sliding_block__dense_activation_silu__prompt'

def setup_inputs():
    _rng = _Rng(jax.random.key(int.from_bytes(__import__("os").urandom(4), "little")))
    _w = lambda a: (lambda t: t.astype(jnp.bfloat16) if jnp.issubdtype(t.dtype, jnp.floating) else t)(jnp.asarray(a))

    def _A_setup():
        B, S, D = (1, 2048, 512)
        return {'x': _w((lambda *s: _rng.normal(s) * 0.05)(B, S, D)), 'wqkv': _w((lambda *s: _rng.normal(s) * 0.05)(D, 3 * D)), 'wo': _w((lambda *s: _rng.normal(s) * 0.05)(D, D))}
    _A_in = _A_setup()

    def _B_setup():
        B, S, D, F = (1, 2048, 512, 1792)
        return {'x': _w((lambda *s: _rng.normal(s) * 0.05)(B, S, D)), 'w1': _w((lambda *s: _rng.normal(s) * 0.8)(D, F) * D ** (-0.5)), 'w2': _w((lambda *s: _rng.normal(s) * 0.8)(F, D) * F ** (-0.5))}
    _B_in = _B_setup()
    return {'A_x': _A_in['x'], 'A_wqkv': _A_in['wqkv'], 'A_wo': _A_in['wo'], 'B_x': _B_in['x'], 'B_w1': _B_in['w1'], 'B_w2': _B_in['w2'], 'c': _w((lambda *s: _rng.normal(s) * 0.05)(1, 512) * 8.0), 'w_mod': _w((lambda *s: _rng.normal(s) * 0.05)(512, 6 * 512) * 512 ** (-0.5) * 8.0)}

def reference(A_x, A_wqkv, A_wo, B_x, B_w1, B_w2, c, w_mod):

    def _A_ref(x, wqkv, wo):
        B, S, D = x.shape
        H = 32
        Dh = D // H
        W = 256
        qkv = (lambda x, *d: x.transpose(*d))((x @ wqkv).reshape(B, S, 3, H, Dh), 2, 0, 3, 1, 4)
        q, k, v = (qkv[0], qkv[1], qkv[2])
        scores = jnp.einsum('bhqd,bhkd->bhqk', q, k) * Dh ** (-0.5)
        idx = jnp.arange(S)
        mask = (idx[:, None] - idx[None, :] >= 0) & (idx[:, None] - idx[None, :] < W)
        scores = jnp.where(mask[None, None], scores, -1000000000.0)
        p = _softmax(scores, axis=-1)
        o = jnp.einsum('bhqk,bhkd->bhqd', p, v)
        return (lambda x, *d: x.transpose(*d))(o, 0, 2, 1, 3).reshape(B, S, D) @ wo

    def _B_ref(x, w1, w2):
        h = jnp.einsum('bsd,df->bsf', x, w1)
        h = _silu(h)
        out = jnp.einsum('bsf,fd->bsd', h, w2)
        return out
    x = A_x
    mod = (_silu(c) @ w_mod).reshape(c.shape[0], 6, 1, -1)
    sa, ca, ga, sb, cb, gb = (mod[:, 0].copy(), mod[:, 1].copy(), mod[:, 2].copy(), mod[:, 3].copy(), mod[:, 4].copy(), mod[:, 5].copy())
    h = _layernorm(x, axis=-1) * (1 + ca) + sa
    x = x + ga * _A_ref(h, A_wqkv, A_wo)
    h = _layernorm(x, axis=-1) * (1 + cb) + sb
    x = x + gb * _B_ref(h, B_w1, B_w2)
    return x
```

```python
import functools
import jax
import jax.numpy as jnp
from jax import lax
import jax.experimental.pallas as pl
import jax.experimental.pallas.tpu as pltpu

S, D, H, DH, WIN, F = 2048, 512, 32, 16, 256, 1792
TQ = 256
NT_STEPS = S // TQ
EPS = 1e-5
QSCALE = (DH ** -0.5) * 1.4426950408889634
NEG = -1e30
LAG = 3
bf16, u32, f32 = jnp.bfloat16, jnp.uint32, jnp.float32
NT_DIMS = (((1,), (1,)), ((), ()))


def _iota(shape, dim):
    return lax.broadcasted_iota(jnp.int32, shape, dim)


def _ln(x):
    m = jnp.mean(x, axis=-1, keepdims=True)
    xc = x - m
    v = jnp.mean(xc * xc, axis=-1, keepdims=True)
    return xc * lax.rsqrt(v + EPS)


def _kernel(x_ref, wqkv_ref, wo_ref, w1_ref, w2_ref, c_ref, wmod_ref, o_ref,
            mod_ref, wqvt_ref, qt_ref, kp_ref, ka_ref, kb_ref, vt_ref, p_ref):
    i = pl.program_id(0)

    @pl.when(i == 0)
    def _():
        c = c_ref[...].astype(f32)
        sc = c * jax.nn.sigmoid(c)
        sc = jnp.broadcast_to(sc, (16, D)).astype(bf16)
        mod_ref[...] = jnp.dot(sc, wmod_ref[...], preferred_element_type=f32)[0:8]
        wt = wqvt_ref.bitcast(bf16)
        wt[0:D, :] = wqkv_ref[:, 0:D].astype(f32).T.astype(bf16)
        wt[D:2 * D, :] = wqkv_ref[:, 2 * D:3 * D].astype(f32).T.astype(bf16)
        kp_ref[...] = jnp.zeros_like(kp_ref)
        ka_ref[0:128, :] = jnp.zeros((128, D), u32)
        kb_ref[0:128, :] = jnp.zeros((128, D), u32)
        vt_ref[0] = jnp.zeros((D // 2, TQ), u32)

    def modv(k):
        return mod_ref[0:1, k * D:(k + 1) * D]

    x = x_ref[...].astype(f32)
    h = (_ln(x) * (1.0 + modv(1)) + modv(0)).astype(bf16)

    kp_ref[0:32, :] = kp_ref[128:160, :]
    kp_ref.bitcast(bf16)[64:320, :] = jnp.dot(
        h, wqkv_ref[:, D:2 * D], preferred_element_type=f32).astype(bf16)
    odd = (_iota((128, D), 1) // DH) % 2 == 1
    k_old = kp_ref[0:128, :]
    k_new = kp_ref[32:160, :]
    r0 = pl.multiple_of(i * 128 + 96, 32)
    ka_ref[pl.ds(r0, 128), :] = jnp.where(odd, k_new, k_old)
    kb_ref[pl.ds(r0, 128), :] = jnp.where(odd, k_old, k_new)
    qv = lax.dot_general(pltpu.bitcast(wqvt_ref[...], bf16), h, NT_DIMS,
                         preferred_element_type=f32)
    qt_ref.bitcast(bf16)[...] = (qv[0:D] * QSCALE).astype(bf16)
    vt_ref.bitcast(bf16)[i + 1] = qv[D:2 * D].astype(bf16)

    lane16 = _iota((16, 128), 1)
    row16 = _iota((16, 128), 0)
    tri64 = _iota((64, 128), 0) > (_iota((64, 128), 1) % 64)
    lo8 = _iota((8, 128), 1) < 64
    lo1 = _iota((1, 128), 1) < 64
    lo32 = _iota((32, 128), 1) < 64
    lo128 = _iota((128, 128), 1) < 64
    pb_ref = p_ref.bitcast(bf16)
    tiles = [(qb, g, j) for qb in range(TQ // 128) for g in range(4) for j in range(8)]
    order = [0, 16, 1, 17, 4, 2, 18, 3, 19, 5, 6, 7, 8, 9, 10, 11, 12, 13, 14, 15]

    def qk(n):
        qb, g, j = tiles[n]
        h_lo, h_hi = g * 8 + j, g * 8 + (j + 1) % 8
        a = qt_ref[h_lo * 8:(h_lo + 1) * 8, qb * 128:(qb + 1) * 128]
        b = qt_ref[h_hi * 8:(h_hi + 1) * 8, qb * 128:(qb + 1) * 128]
        parts = [jnp.zeros((8, 128), u32)] * 8
        parts[j] = jnp.where(lo8, a, u32(0))
        parts[(j + 1) % 8] = jnp.where(lo8, u32(0), b)
        ww = pltpu.bitcast(jnp.concatenate(parts, axis=0), bf16)
        krow0 = pl.multiple_of(i * 128 + qb * 64, 64)
        kk = (ka_ref if j % 2 == 0 else kb_ref)[pl.ds(krow0, 160), g * 128:(g + 1) * 128]
        X = {}
        for s_ in range(4):
            gg = order[s_ * 5:(s_ + 1) * 5]
            lhs = pltpu.bitcast(jnp.concatenate([kk[c * 8:(c + 1) * 8] for c in gg], axis=0), bf16)
            s = jnp.dot(lhs, ww, preferred_element_type=f32)
            for n_, c in enumerate(gg):
                X[c] = s[n_ * 16:(n_ + 1) * 16]
        kmin = 256 - (i * TQ + qb * 128) - (lane16 // 64) * 64
        ch = []
        for c in range(16):
            v = jnp.where(row16 + c * 16 >= kmin, X[c], NEG)
            if c < 4:
                v = jnp.where((row16 + c * 16) > (lane16 % 64), v, X[16 + c])
            ch.append(v)
        return jnp.concatenate(ch, axis=0)

    def sm(n, s2):
        m = jnp.max(s2, axis=0, keepdims=True)
        p = jnp.exp2(s2 - m)
        l = jnp.sum(p, axis=0, keepdims=True)
        pm = p[0:64]
        pf = jnp.concatenate([jnp.where(tri64, pm, 0.), p[64:256], jnp.where(tri64, 0., pm)], axis=0)
        pb_ref[:, (n % 16) * 128:(n % 16 + 1) * 128] = pf.astype(bf16)
        return l

    def pv(n_lo, n_hi, l_lo, l_hi):
        qb, g, j = tiles[n_lo]
        hh = g * 8 + j
        X = p_ref[:, (n_lo % 16) * 128:(n_lo % 16 + 1) * 128]
        Y = p_ref[:, (n_hi % 16) * 128:(n_hi % 16 + 1) * 128]
        pt = jnp.concatenate([jnp.where(lo32, X[0:32], u32(0)),
                              jnp.where(lo128, X[32:160], Y[0:128]),
                              jnp.where(lo32, u32(0), Y[128:160])], axis=0)
        vparts = []
        for c in range(3):
            kb = qb + c
            vparts.append(vt_ref[i + kb // 2, hh * 8:(hh + 1) * 8, (kb % 2) * 128:(kb % 2 + 1) * 128])
        vt = pltpu.bitcast(jnp.concatenate(vparts, axis=1), bf16)
        o = jnp.dot(vt, pltpu.bitcast(pt, bf16), preferred_element_type=f32)
        l = jnp.where(lo1, l_lo, l_hi)
        return o * pl.reciprocal(l, approx=True)

    N = len(tiles)
    pend = {n: qk(n) for n in range(LAG)}
    ls, ot = {}, {}
    ob = {}
    for n in range(N):
        if n + LAG < N:
            pend[n + LAG] = qk(n + LAG)
        ls[n] = sm(n, pend.pop(n))
        j = n % 8
        if j > 0:
            ot[n] = pv(n, n - 1, ls[n], ls[n - 1])
        if j == 7:
            ot[n - 7] = pv(n - 7, n, ls[n - 7], ls[n])
            ob[n // 8] = jnp.concatenate([ot.pop(k) for k in range(n - 7, n + 1)], axis=0).T
    o = jnp.concatenate([jnp.concatenate([ob[qb * 4 + g] for g in range(4)], axis=1)
                         for qb in range(TQ // 128)], axis=0).astype(bf16)

    x1 = x + modv(2) * jnp.dot(o, wo_ref[...], preferred_element_type=f32)
    h2 = (_ln(x1) * (1.0 + modv(4)) + modv(3)).astype(bf16)
    z = jnp.dot(h2, w1_ref[...], preferred_element_type=f32)
    hz = 0.5 * z
    a = (hz + hz * jnp.tanh(hz)).astype(bf16)
    y = jnp.dot(a, w2_ref[...], preferred_element_type=f32)
    o_ref[...] = (x1 + modv(5) * y).astype(o_ref.dtype)


@jax.jit
def pallas_adaLN_cond__sliding_block__dense_activation_silu__prompt_kernel(
        A_x, A_wqkv, A_wo, B_x, B_w1, B_w2, c, w_mod):
    del B_x
    x = A_x.reshape(S, D)
    full = lambda shp: pl.BlockSpec(shp, lambda i: (0,) * len(shp))
    out = pl.pallas_call(
        _kernel,
        grid=(NT_STEPS,),
        in_specs=[pl.BlockSpec((TQ, D), lambda i: (i, 0)), full((D, 3 * D)), full((D, D)),
                  full((D, F)), full((F, D)), full((1, D)), full((D, 6 * D))],
        out_specs=pl.BlockSpec((TQ, D), lambda i: (i, 0)),
        out_shape=jax.ShapeDtypeStruct((S, D), A_x.dtype),
        scratch_shapes=[
            pltpu.VMEM((8, 6 * D), f32),
            pltpu.VMEM((D, D), u32),
            pltpu.VMEM((D // 2, TQ), u32),
            pltpu.VMEM((160, D), u32),
            pltpu.VMEM(((S + 256) // 2, D), u32),
            pltpu.VMEM(((S + 256) // 2, D), u32),
            pltpu.VMEM((NT_STEPS + 1, D // 2, TQ), u32),
            pltpu.VMEM((160, 16 * 128), u32),
        ],
        compiler_params=pltpu.CompilerParams(
            dimension_semantics=("arbitrary",), vmem_limit_bytes=100 * 1024 * 1024),
    )(x, A_wqkv, A_wo, B_w1, B_w2, c, w_mod)
    return out.reshape(1, S, D)
```

```python
import functools

import jax
import jax.numpy as jnp
from jax import lax
import jax.experimental.pallas as pl
import jax.experimental.pallas.tpu as pltpu

S, D, DH, F = 2048, 512, 16, 1792
TQ = 256
NTILES = S // TQ
NFC = F // 128
EPS = 1e-5
QSCALE = (DH ** -0.5) * 1.4426950408889634
NEG = -1e30
NS = 4
SB = 128 // NS
CB = SB // 16
NCH = 16 + CB
KW = (384 + SB) // 2
KC = (128 - SB) // 2
NPS = 32
bf16, u32, f32 = jnp.bfloat16, jnp.uint32, jnp.float32
NT_DIMS = (((1,), (1,)), ((), ()))
TILES = [(qb, g, j) for qb in range(TQ // 128) for g in range(4) for j in range(8)]
N = len(TILES)


def _iota(shape, dim):
    return lax.broadcasted_iota(jnp.int32, shape, dim)


def _ln(x):
    xc = x - jnp.mean(x, axis=-1, keepdims=True)
    ss = jnp.sum(xc * xc, axis=-1, keepdims=True) + D * EPS
    return xc * jnp.exp2(-0.5 * jnp.log2(ss))


def _modulate(n, scale, shift):
    return (n * ((1.0 + scale) * D ** 0.5) + shift).astype(bf16)


def _silu(z):
    hz = 0.5 * z
    return hz + hz * jnp.tanh(hz)


def _dot(a, b):
    return jnp.dot(a, b, preferred_element_type=f32)


def _as_bf16(x):
    return pltpu.bitcast(x, bf16)


def _cols(c):
    return slice(c * 128, (c + 1) * 128)


def _lane_select(pieces, zero):
    keys = sorted(pieces)
    grp = _iota(pieces[keys[0]].shape, 1) // SB
    v = pieces[keys[0]]
    for a in keys[1:]:
        v = jnp.where(grp >= a, pieces[a], v)
    if keys[0] > 0:
        v = jnp.where(grp >= keys[0], v, zero)
    if keys[-1] < NS - 1:
        v = jnp.where(grp >= keys[-1] + 1, zero, v)
    return v


def _tree(op, xs):
    while len(xs) > 1:
        xs = [op(xs[k], xs[k + 1]) if k + 1 < len(xs) else xs[k] for k in range(0, len(xs), 2)]
    return xs[0]


def _col_max(groups):
    ms = []
    for grp in groups:
        halves = [h for v in grp for h in (v[0:8], v[8:16])]
        ms.append(functools.reduce(jnp.maximum, halves))
    return jnp.max(_tree(jnp.maximum, ms), axis=0, keepdims=True)


def _col_sum(p):
    accs = [None, None]
    for k in range(p.shape[0] // 16):
        v = p[k * 16:k * 16 + 8] + p[k * 16 + 8:k * 16 + 16]
        accs[k % 2] = v if accs[k % 2] is None else accs[k % 2] + v
    return jnp.sum(accs[0] + accs[1], axis=0, keepdims=True)


class _Heads:
    def __init__(self):
        self.ot, self.ob = {}, {}

    def add(self, k, o):
        self.ot[k] = o
        ks = range(k // 8 * 8, k // 8 * 8 + 8)
        if all(kk in self.ot for kk in ks):
            self.ob[k // 8] = jnp.concatenate([self.ot[kk] for kk in ks], axis=0).T

    def result(self):
        return jnp.concatenate(
            [jnp.concatenate([self.ob[qb * 4 + g] for g in range(4)], axis=1)
             for qb in range(TQ // 128)], axis=0)


def _kernel(x_hbm, wqkv_hbm, wo_hbm, w1_hbm, w2_hbm, c_hbm, wmod_hbm, o_hbm,
            x_v, wqkv_v, wo_v, w1_v, w2_v, c_v, wmod_v,
            mod_ref, wqvt_ref, qt_ref, q0_ref, kp_ref, k01_ref, kw_ref, vt_ref, p_ref,
            x1_ref, h2_ref, h01_ref, n_ref, acc_ref, a_ref, sc_ref, cnt_ref, sems, osems):
    def cp(src, dst, idx, k):
        return pltpu.make_async_copy(src.at[idx], dst.at[idx], sems.at[k])
    al = slice(None)
    mparts = [(0, 256), (256, 384), (384, 512)]
    d_c = cp(c_hbm, c_v, (al, al), 0)
    d_x01 = cp(x_hbm, x_v, (slice(0, 2 * TQ), al), 1)
    d_m = [[cp(wmod_hbm, wmod_v, (al, slice(k * D + a, k * D + b)), 2 + 2 * i + k) for k in range(2)]
           for i, (a, b) in enumerate(mparts)]
    d_qk = [cp(wqkv_hbm, wqkv_v, (_cols(j), slice(0, 2 * D)), 8 + j) for j in range(4)]
    d_wv = cp(wqkv_hbm, wqkv_v, (al, slice(2 * D, 3 * D)), 12)
    d_wo = cp(wo_hbm, wo_v, (al, al), 13)
    d_mb = cp(wmod_hbm, wmod_v, (al, slice(2 * D, 6 * D)), 14)
    d_w1 = cp(w1_hbm, w1_v, (al, al), 15)
    d_w2 = cp(w2_hbm, w2_v, (al, al), 16)
    d_x2 = cp(x_hbm, x_v, (slice(2 * TQ, 3 * TQ), al), 17)
    d_xr = cp(x_hbm, x_v, (slice(3 * TQ, S), al), 18)
    for d in ([d_c, d_x01] + d_m[0] + [d_qk[0]] + d_m[1] + [d_qk[1]] + d_m[2]
              + [d_qk[2], d_qk[3], d_wv, d_wo, d_mb, d_x2, d_w1, d_w2, d_xr]):
        d.start()

    def rows_of(t):
        return pl.ds(t * TQ if isinstance(t, int) else pl.multiple_of(t * TQ, TQ), TQ)

    def out_copy(t):
        return pltpu.make_async_copy(x_v.at[rows_of(t)], o_hbm.at[rows_of(t)], osems.at[t])

    def modv(k):
        return mod_ref[0:1, k * D:(k + 1) * D]

    def mod_cols(a, b):
        mod_ref[:, a:b] = _dot(sc_ref[...].astype(bf16), wmod_v[:, a:b])[0:8]

    def ln1(t):
        return _modulate(_ln(x_v[rows_of(t), :].astype(f32)), modv(1), modv(0))

    def build_windows(src_ref, dst0, nrows, alt=False):
        lane = _iota((nrows, 128), 1) & (DH * NS - 1)
        ge = (lambda i: lane > DH * i - 1) if alt else (lambda i: lane >= DH * i)
        for g in range(4):
            ks = [src_ref[o * SB // 2:o * SB // 2 + nrows, _cols(g)] for o in range(NS)]
            for v in range(NS):
                val = ks[(0 - v) % NS]
                for i in range(1, NS):
                    val = jnp.where(ge(i), ks[(i - v) % NS], val)
                kw_ref[v, dst0:dst0 + nrows, _cols(g)] = val

    def advance_windows():
        for v in range(NS):
            kw_ref[v, 0:KW - 128, :] = kw_ref[v, 128:KW, :]
        build_windows(kp_ref, KW - 128, 128)

    def k_tasks(get_h):
        def run(c):
            if c == 0:
                kp_ref[0:KC, :] = kp_ref[128:128 + KC, :]
            kp_ref.bitcast(bf16)[2 * KC:2 * KC + TQ, _cols(c)] = _dot(
                get_h(), wqkv_v[:, _cols(4 + c)]).astype(bf16)
        return [functools.partial(run, c) for c in range(4)]

    def t_dot(r0, r1, h):
        return lax.dot_general(_as_bf16(wqvt_ref[r0 // 2:r1 // 2, :]), h, NT_DIMS,
                               preferred_element_type=f32)

    def attention_first(tail):
        lane16, row16 = _iota((16, 128), 1), _iota((16, 128), 0)

        def scores(n):
            qb, g, j = TILES[n]
            parts = [jnp.zeros((8, 128), u32)] * 8
            parts[j] = q0_ref[(g * 8 + j) * 8:(g * 8 + j + 1) * 8, _cols(qb)]
            ww = _as_bf16(jnp.concatenate(parts, axis=0))
            groups = []
            for c0 in range(0, 8 * qb + 8, 4):
                s = _dot(_as_bf16(k01_ref[c0 * 8:(c0 + 4) * 8, _cols(g)]), ww)
                grp = [s[k * 16:(k + 1) * 16] for k in range(4)]
                if c0 >= 8 * qb:
                    grp = [jnp.where(row16 + (c0 + k - 8 * qb) * 16 > lane16, NEG, v)
                           for k, v in enumerate(grp)]
                groups.append(grp)
            p = jnp.exp2(jnp.concatenate(sum(groups, []), axis=0) - _col_max(groups))
            return p, _col_sum(p)

        heads, st, nq = _Heads(), {}, 0
        for n in range(N):
            while nq < N and nq <= n + (7, 5)[TILES[nq][0]]:
                st[nq] = scores(nq)
                nq += 1
            qb, g, j = TILES[n]
            p, l = st.pop(n)
            vt = vt_ref[(g * 8 + j) * 8:(g * 8 + j + 1) * 8, 0:(qb + 1) * 128]
            heads.add(n, _dot(_as_bf16(vt), p.astype(bf16)) * pl.reciprocal(l, approx=True))
            if N - 1 - n in tail:
                tail[N - 1 - n]()
        return heads.result()

    def attention(fillers, tail, tail_pos):
        lane16, row16 = _iota((16, 128), 1), _iota((16, 128), 0)
        tri = _iota((SB, 128), 0) > (_iota((SB, 128), 1) % SB)
        grp8 = _iota((8, 128), 1) // SB
        order = [c for k in range(CB) for c in (k, 16 + k)] + list(range(CB, 16))
        splits = [order[0:5], order[5:9], order[9:14], order[14:18]]
        slot = lambda n: _cols(n % NPS)

        def scores(n):
            qb, g, j = TILES[n]
            parts = [jnp.zeros((8, 128), u32)] * 8
            for a in range(NS):
                hh = g * 8 + (j + a) % 8
                q = qt_ref[hh * 8:(hh + 1) * 8, _cols(qb)]
                if a == 0:
                    q = jnp.where(grp8 >= 1, u32(0), q)
                elif a == NS - 1:
                    q = jnp.where(grp8 >= a, q, u32(0))
                else:
                    q = jnp.where(grp8 == a, q, u32(0))
                parts[(j + a) % 8] = q
            ww = _as_bf16(jnp.concatenate(parts, axis=0))
            X = {}
            for gg in splits:
                lhs = jnp.concatenate(
                    [kw_ref[j % NS, qb * 64 + c * 8:qb * 64 + (c + 1) * 8, _cols(g)] for c in gg], axis=0)
                s = _dot(_as_bf16(lhs), ww)
                for k, c in enumerate(gg):
                    X[c] = s[k * 16:(k + 1) * 16]
            for c in range(CB):
                X[c] = jnp.where((row16 + c * 16) > (lane16 % SB), X[c], X[16 + c])
            m = _col_max([[X[c % 16] for c in gg if c >= CB] for gg in splits])
            p = jnp.exp2(jnp.concatenate([X[c] for c in range(16)], axis=0) - m)
            pm = p[0:SB]
            p_ref.bitcast(bf16)[:, slot(n)] = jnp.concatenate(
                [jnp.where(tri, pm, 0.), p[SB:256], jnp.where(tri, 0., pm)], axis=0).astype(bf16)
            return _col_sum(p)

        def pv(n):
            qb, g, j = TILES[n]
            src = [n - j + (j - a) % 8 for a in range(NS)]
            parts = []
            for t in range(0, 24, CB):
                parts.append(_lane_select(
                    {a: p_ref[(t - CB * a) * 8:(t - CB * a + CB) * 8, slot(src[a])]
                     for a in range(NS) if 0 <= t - CB * a < NCH}, u32(0)))
            vt = vt_ref[(g * 8 + j) * 8:(g * 8 + j + 1) * 8, qb * 128:qb * 128 + 384]
            o = _dot(_as_bf16(vt), _as_bf16(jnp.concatenate(parts, axis=0)))
            l = _lane_select({a: ls[src[a]] for a in range(NS)}, 0.)
            heads.add(n, o * pl.reciprocal(l, approx=True))

        pv_at = {(n if n % 8 >= NS - 1 else n + 8): n for n in range(N)}
        heads, ls, fillers = _Heads(), {}, list(fillers)
        nq, npv, nf = 0, -4, -2
        while npv < N + 8:
            for tok in "QFQPP":
                if tok == "Q" and nq < N:
                    ls[nq] = scores(nq)
                    nq += 1
                elif tok == "P":
                    if npv == N - tail_pos:
                        tail()
                    if npv in pv_at:
                        pv(pv_at[npv])
                    npv += 1
                elif tok == "F":
                    if nf >= 0 and fillers:
                        fillers.pop(0)()
                    nf += 1
        assert not fillers
        return heads.result()

    def out_proj(t, o, mix=None):
        ys = []
        for r in range(0, TQ, 128):
            ob = o[r:r + 128].astype(bf16)
            if mix is None:
                ys.append(_dot(ob, wo_v[...]))
            else:
                cols = []
                for c in range(4):
                    cols.append(_dot(ob, wo_v[:, _cols(c)]))
                    for fl in mix.pop(0):
                        fl()
                ys.append(jnp.concatenate(cols, axis=1))
        x1 = x_v[rows_of(t), :].astype(f32) + modv(2) * jnp.concatenate(ys, axis=0)
        return x1, _modulate(_ln(x1), modv(4), modv(3))

    def h2_half(r):
        return _as_bf16(h2_ref[r * 64:(r + 1) * 64, :])

    def finish(t, c, x1, y):
        x_v[rows_of(t), _cols(c)] = (x1 + mod_ref[0:1, _cols(20 + c)] * y).astype(bf16)

    def ffn1_tasks():
        def run(c, r):
            a_ref.bitcast(bf16)[r * 128:(r + 1) * 128, _cols(c)] = _silu(
                _dot(h2_half(r), w1_v[:, _cols(c)])).astype(bf16)
        return [functools.partial(run, c, r) for c in range(NFC) for r in range(2)]

    def ffn2(t, c):
        finish(t, c, x1_ref[:, _cols(c)], _dot(_as_bf16(a_ref[...]), w2_v[:, _cols(c)]))
        x1_ref[:, _cols(c)] = n_ref[0:TQ, _cols(c)]

    def ffn_value_tasks(get_h2, get_x1, t, early):
        acts, accs = {}, {}

        def run1(c, r):
            acts[(c, r)] = _silu(_dot(get_h2(r), w1_v[:, _cols(c)]))

        def run2(c, k0, k1):
            a = jnp.concatenate(
                [jnp.concatenate([acts[(k, r)] for k in range(k0, k1)], axis=1) for r in range(2)],
                axis=0).astype(bf16)
            y = _dot(a, w2_v[k0 * 128:k1 * 128, _cols(c)])
            if k0 > 0:
                y = y + accs.pop(c)
            if k1 < NFC:
                accs[c] = y
            else:
                finish(t, c, get_x1(c), y)

        t1 = [functools.partial(run1, c, r) for c in range(NFC) for r in range(2)]
        if not early:
            return t1, [functools.partial(run2, c, 0, NFC) for c in range(4)]
        for c in range(4):
            t1.insert(12 + c * 5, functools.partial(run2, c, 0, 4))
        return t1, [functools.partial(run2, c, 4, NFC) for c in range(4)]

    def mid_step(s, get_h, fill):
        def proj_q():
            qt_ref.bitcast(bf16)[...] = (t_dot(0, D, get_h()) * QSCALE).astype(bf16)
        o = attention(fill, proj_q, 1)
        advance_windows()
        x1, h2 = out_proj(s, o)
        h2_ref.bitcast(bf16)[...] = h2
        n_ref[0:TQ, :] = x1
        vt_ref[:, 0:TQ] = vt_ref[:, TQ:2 * TQ]
        vt_ref.bitcast(bf16)[:, TQ:2 * TQ] = t_dot(D, 2 * D, get_h()).astype(bf16)

    def once(fn):
        def body(i, carry):
            fn()
            return carry
        lax.fori_loop(1, cnt_ref[0], body, 0)

    cnt_ref[0] = 2
    d_c.wait()
    c = c_v[...].astype(f32)
    sc_ref[...] = jnp.broadcast_to(c * jax.nn.sigmoid(c), (16, D))
    d_x01.wait()
    n_ref[...] = _ln(x_v[0:2 * TQ, :].astype(f32))
    ha = lambda: _as_bf16(h01_ref[0:TQ // 2, :])
    hb = lambda: _as_bf16(h01_ref[TQ // 2:TQ, :])
    wt = wqvt_ref.bitcast(bf16)

    def h_cols(i):
        a, b = mparts[i]
        mod_cols(a, b)
        mod_cols(D + a, D + b)
        h01_ref.bitcast(bf16)[:, a:b] = _modulate(
            n_ref[:, a:b], mod_ref[0:1, D + a:D + b], mod_ref[0:1, a:b])

    for d in d_m[0]:
        d.wait()
    h_cols(0)
    for j in range(4):
        d_qk[j].wait()
        for d in (d_m[j] if j in (1, 2) else [d_wv] if j == 3 else []):
            d.wait()
        hj = _as_bf16(h01_ref[:, _cols(j)])
        ya = _dot(hj, wqkv_v[_cols(j), 0:D])
        if j in (1, 2):
            h_cols(j)
        y = jnp.concatenate([ya, _dot(hj, wqkv_v[_cols(j), D:2 * D])], axis=1)
        if j > 0:
            y = y + acc_ref[...]
        if j < 3:
            acc_ref[...] = y
        wt[0:D, _cols(j)] = wqkv_v[_cols(j), 0:D].astype(f32).T.astype(bf16)
    q0_ref.bitcast(bf16)[...] = (y[0:TQ, 0:D] * QSCALE).T.astype(bf16)
    qt_ref.bitcast(bf16)[...] = (y[TQ:2 * TQ, 0:D] * QSCALE).T.astype(bf16)
    k01_ref.bitcast(bf16)[...] = y[:, D:2 * D].astype(bf16)
    build_windows(k01_ref, 0, KW, alt=True)
    kp_ref[128:128 + KC, :] = k01_ref[TQ - KC:TQ, :]
    vt_ref.bitcast(bf16)[:, 0:TQ] = _dot(ha(), wqkv_v[:, 2 * D:3 * D]).T.astype(bf16)
    wt[D:2 * D, :] = wqkv_v[:, 2 * D:3 * D].astype(f32).T.astype(bf16)

    def v1(r, half):
        vt_ref.bitcast(bf16)[_cols(r), _cols(2 + half)] = t_dot(
            D + r * 128, D + (r + 1) * 128, hb()[_cols(half)]).astype(bf16)
    v1s = [functools.partial(v1, r, half) for r in range(4) for half in range(2)]
    o0 = attention_first(dict(zip((4, 2, 1, 0), v1s[:4])))
    d_wo.wait()
    d_mb.wait()
    d_x2.wait()

    def finish_tile0():
        m = [functools.partial(mod_cols, 2 * D + k * 128, 2 * D + (k + 1) * 128) for k in range(16)]
        h01_ref.bitcast(bf16)[0:TQ, :] = ln1(2)
        k = k_tasks(ha)
        x1, h2 = out_proj(0, o0, [
            [m[0]], [m[1]], [m[2]], [m[3], k[0], m[4], m[5], k[1], m[6], m[7]],
            [m[8]], [m[9]], [m[10]], [m[11], k[2], m[12], m[13], m[14], m[15], k[3]]])
        x1_ref[...] = x1
        h2_ref.bitcast(bf16)[...] = h2
    once(finish_tile0)

    d_w1.wait()
    once(lambda: mid_step(1, ha, v1s[4:] + ffn1_tasks()))
    d_w2.wait()
    d_xr.wait()

    def body(s, carry):
        ffn2(s - 2, 0)
        ffn2(s - 2, 1)
        h = ln1(s + 1)
        ffn2(s - 2, 2)
        ffn2(s - 2, 3)
        out_copy(s - 2).start()
        mid_step(s, lambda: h, ffn1_tasks() + k_tasks(lambda: h))
        return carry

    lax.fori_loop(2, NTILES - 1, body, 0)

    t = NTILES - 1
    for c in range(4):
        ffn2(t - 2, c)
    out_copy(t - 2).start()
    fill, rest = ffn_value_tasks(h2_half, lambda c: x1_ref[:, _cols(c)], t - 1, True)
    o = attention(fill, rest[0], -7)
    rest[1]()
    x1, h2 = out_proj(t, o)
    rest[2]()
    rest[3]()
    out_copy(t - 1).start()
    t1, t2 = ffn_value_tasks(lambda r: h2[_cols(r)], lambda c: x1[:, _cols(c)], t, False)
    for fl in t1:
        fl()

    def last_copy(c):
        idx = (rows_of(t), _cols(c))
        return pltpu.make_async_copy(x_v.at[idx], o_hbm.at[idx], osems.at[t + c])
    for c, fl in enumerate(t2):
        fl()
        last_copy(c).start()
    for k in range(NTILES - 1):
        out_copy(k).wait()
    for c in range(4):
        last_copy(c).wait()


@jax.jit
def pallas_adaLN_cond__sliding_block__dense_activation_silu__prompt_kernel(
        A_x: jax.Array,
        A_wqkv: jax.Array,
        A_wo: jax.Array,
        B_x: jax.Array,
        B_w1: jax.Array,
        B_w2: jax.Array,
        c: jax.Array,
        w_mod: jax.Array,
):
    del B_x
    anyspec = pl.BlockSpec(memory_space=pl.ANY)
    out = pl.pallas_call(
        _kernel,
        in_specs=[anyspec] * 7,
        out_specs=anyspec,
        out_shape=jax.ShapeDtypeStruct((S, D), A_x.dtype),
        scratch_shapes=[
            pltpu.VMEM((S, D), bf16),
            pltpu.VMEM((D, 3 * D), bf16),
            pltpu.VMEM((D, D), bf16),
            pltpu.VMEM((D, F), bf16),
            pltpu.VMEM((F, D), bf16),
            pltpu.VMEM((1, D), bf16),
            pltpu.VMEM((D, 6 * D), bf16),
            pltpu.VMEM((8, 6 * D), f32),
            pltpu.VMEM((D, D), u32),
            pltpu.VMEM((D // 2, TQ), u32),
            pltpu.VMEM((D // 2, TQ), u32),
            pltpu.VMEM((KC + 128, D), u32),
            pltpu.VMEM((TQ, D), u32),
            pltpu.VMEM((NS, KW, D), u32),
            pltpu.VMEM((D // 2, 2 * TQ), u32),
            pltpu.VMEM((NCH * 8, NPS * 128), u32),
            pltpu.VMEM((TQ, D), f32),
            pltpu.VMEM((TQ // 2, D), u32),
            pltpu.VMEM((TQ, D), u32),
            pltpu.VMEM((2 * TQ, D), f32),
            pltpu.VMEM((2 * TQ, 2 * D), f32),
            pltpu.VMEM((TQ // 2, F), u32),
            pltpu.VMEM((16, D), f32),
            pltpu.SMEM((1,), jnp.int32),
            pltpu.SemaphoreType.DMA((19,)),
            pltpu.SemaphoreType.DMA((NTILES + 3,)),
        ],
        compiler_params=pltpu.CompilerParams(vmem_limit_bytes=64 * 1024 * 1024),
    )(A_x.reshape(S, D), A_wqkv, A_wo, B_w1, B_w2, c, w_mod)
    return out.reshape(1, S, D)
```

```python
import functools

import jax
import jax.numpy as jnp
from jax import lax
import jax.experimental.pallas as pl
import jax.experimental.pallas.tpu as pltpu

S, D, DH, F = 2048, 512, 16, 1792
TQ = 256
NTILES = S // TQ
NFC = F // 128
EPS = 1e-5
QSCALE = (DH ** -0.5) * 1.4426950408889634
NEG = -1e30
NS = 4
SB = 128 // NS
CB = SB // 16
NCH = 16 + CB
KW = (384 + SB) // 2
KC = (128 - SB) // 2
NPS = 32
bf16, u32, f32 = jnp.bfloat16, jnp.uint32, jnp.float32
NT_DIMS = (((1,), (1,)), ((), ()))
TILES = [(qb, g, j) for qb in range(TQ // 128) for g in range(4) for j in range(8)]
N = len(TILES)


def _iota(shape, dim):
    return lax.broadcasted_iota(jnp.int32, shape, dim)


def _ln(x):
    xc = x - jnp.mean(x, axis=-1, keepdims=True)
    ss = jnp.sum(xc * xc, axis=-1, keepdims=True) + D * EPS
    return xc * jnp.exp2(-0.5 * jnp.log2(ss))


def _modulate(n, scale, shift):
    return (n * ((1.0 + scale) * D ** 0.5) + shift).astype(bf16)


def _silu(z):
    hz = 0.5 * z
    return hz + hz * jnp.tanh(hz)


def _dot(a, b):
    return jnp.dot(a, b, preferred_element_type=f32)


def _as_bf16(x):
    return pltpu.bitcast(x, bf16)


def _cols(c):
    return slice(c * 128, (c + 1) * 128)


def _tree(op, xs):
    while len(xs) > 1:
        xs = [op(xs[k], xs[k + 1]) if k + 1 < len(xs) else xs[k] for k in range(0, len(xs), 2)]
    return xs[0]


def _col_max(blocks):
    ms = [functools.reduce(lax.max, [b[k:k + 8] for k in range(0, b.shape[0], 8)]) for b in blocks]
    return jnp.max(_tree(lax.max, ms), axis=0, keepdims=True)


def _col_sum(p):
    p = p.reshape(-1, 2, 2, 8, 128)
    v = jnp.sum(p[:, :, 0] + p[:, :, 1], axis=0)
    return jnp.sum(v[0] + v[1], axis=0, keepdims=True)


class _Heads:
    def __init__(self):
        self.ot, self.ob = {}, {}

    def add(self, k, o):
        self.ot[k] = o
        ks = range(k // 8 * 8, k // 8 * 8 + 8)
        if all(kk in self.ot for kk in ks):
            self.ob[k // 8] = jnp.concatenate([self.ot[kk] for kk in ks], axis=0).T

    def result(self):
        return jnp.concatenate(
            [jnp.concatenate([self.ob[qb * 4 + g] for g in range(4)], axis=1)
             for qb in range(TQ // 128)], axis=0)


def _kernel(x_hbm, wqkv_hbm, wo_hbm, w1_hbm, w2_hbm, c_hbm, wmod_hbm, o_hbm,
            x_v, wqkv_v, wo_v, w1_v, w2_v, c_v, wmod_v,
            mod_ref, wqvt_ref, qt_ref, q0_ref, kp_ref, k01_ref, kw_ref, vt_ref, p_ref,
            x1_ref, h2_ref, h01_ref, n_ref, acc_ref, a_ref, sc_ref, cnt_ref, sems):
    def cp(src, dst, idx, k):
        return pltpu.make_async_copy(src.at[idx], dst.at[idx], sems.at[k])
    al = slice(None)
    mparts = [(0, 256), (256, 384), (384, 512)]
    d_c = cp(c_hbm, c_v, (al, al), 0)
    d_x01 = cp(x_hbm, x_v, (slice(0, 2 * TQ), al), 0)
    d_m = [[cp(wmod_hbm, wmod_v, (al, slice(k * D + a, k * D + b)), (1, 3, 4)[i]) for k in range(2)]
           for i, (a, b) in enumerate(mparts)]
    d_qk = [cp(wqkv_hbm, wqkv_v, (_cols(j), slice(0, 2 * D)), 2 + j) for j in range(4)]
    d_wv = cp(wqkv_hbm, wqkv_v, (al, slice(2 * D, 3 * D)), 5)
    d_wo = cp(wo_hbm, wo_v, (al, al), 6)
    d_mb = cp(wmod_hbm, wmod_v, (al, slice(2 * D, 6 * D)), 6)
    d_x2 = cp(x_hbm, x_v, (slice(2 * TQ, 3 * TQ), al), 6)
    d_w1 = cp(w1_hbm, w1_v, (al, al), 7)
    d_w2 = cp(w2_hbm, w2_v, (al, al), 8)
    d_xr = cp(x_hbm, x_v, (slice(3 * TQ, S), al), 8)
    for d in ([d_c, d_x01] + d_m[0] + [d_qk[0]] + d_m[1] + [d_qk[1]] + d_m[2]
              + [d_qk[2], d_qk[3], d_wv, d_wo, d_mb, d_x2, d_w1, d_w2, d_xr]):
        d.start()

    def rows_of(t):
        return pl.ds(t * TQ if isinstance(t, int) else pl.multiple_of(t * TQ, TQ), TQ)

    def out_copy(t):
        return pltpu.make_async_copy(x_v.at[rows_of(t)], o_hbm.at[rows_of(t)], sems.at[0])

    def modv(k):
        return mod_ref[0:1, k * D:(k + 1) * D]

    def mod_cols(a, b):
        mod_ref[:, a:b] = _dot(sc_ref[...].astype(bf16), wmod_v[:, a:b])[0:8]

    def ln1(t):
        return _modulate(_ln(x_v[rows_of(t), :].astype(f32)), modv(1), modv(0))

    def build_windows(src_ref, dst0, nrows, alt=False):
        lane = _iota((nrows, 128), 1) & (DH * NS - 1)
        ge = {i: (lane > DH * i - 1) if alt else (lane >= DH * i) for i in range(1, NS)}
        for g in range(4):
            ks = [src_ref[o * SB // 2:o * SB // 2 + nrows, _cols(g)] for o in range(NS)]
            for v in range(NS):
                val = ks[(0 - v) % NS]
                for i in range(1, NS):
                    val = lax.select(ge[i], ks[(i - v) % NS], val)
                kw_ref[v, dst0:dst0 + nrows, _cols(g)] = val

    def advance_windows():
        for v in range(NS):
            kw_ref[v, 0:KW - 128, :] = kw_ref[v, 128:KW, :]
        build_windows(kp_ref, KW - 128, 128)

    def k_tasks(get_h):
        def run(c):
            if c == 0:
                kp_ref[0:KC, :] = kp_ref[128:128 + KC, :]
            kp_ref.bitcast(bf16)[2 * KC:2 * KC + TQ, _cols(c)] = _dot(
                get_h(), wqkv_v[:, _cols(4 + c)]).astype(bf16)
        return [functools.partial(run, c) for c in range(4)]

    def t_dot(r0, r1, h):
        return lax.dot_general(_as_bf16(wqvt_ref[r0 // 2:r1 // 2, :]), h, NT_DIMS,
                               preferred_element_type=f32)

    def attention_first(tail):
        future = [_iota((64, 128), 0) + 64 * k > _iota((64, 128), 1) for k in range(2)]
        neg = jnp.full((64, 128), NEG, f32)
        zero8 = jnp.zeros((8, 128), u32)

        def scores(n):
            qb, g, j = TILES[n]
            parts = [zero8] * 8
            parts[j] = q0_ref[(g * 8 + j) * 8:(g * 8 + j + 1) * 8, _cols(qb)]
            ww = _as_bf16(jnp.concatenate(parts, axis=0))
            blocks = []
            for b in range(2 * qb + 2):
                s = _dot(_as_bf16(k01_ref[b * 32:(b + 1) * 32, _cols(g)]), ww)
                blocks.append(lax.select(future[b - 2 * qb], neg, s) if b >= 2 * qb else s)
            p = jnp.exp2(jnp.concatenate(blocks, axis=0) - _col_max(blocks))
            return p, _col_sum(p)

        heads, st, nq = _Heads(), {}, 0
        for n in range(N):
            while nq < N and nq <= n + (7, 5)[TILES[nq][0]]:
                st[nq] = scores(nq)
                nq += 1
            qb, g, j = TILES[n]
            p, l = st.pop(n)
            vt = vt_ref[(g * 8 + j) * 8:(g * 8 + j + 1) * 8, 0:(qb + 1) * 128]
            heads.add(n, _dot(_as_bf16(vt), p.astype(bf16)) * pl.reciprocal(l, approx=True))
            if N - 1 - n in tail:
                tail[N - 1 - n]()
        return heads.result()

    def attention(fillers, tail, tail_pos):
        tri = _iota((SB, 128), 0) > (_iota((SB, 128), 1) & (SB - 1))
        zero_p = jnp.zeros((SB, 128), f32)
        ge = {(r, a): _iota((r, 128), 1) >= a * SB for r in (1, 8, 16, 96) for a in range(1, NS)}
        eq = {a: (_iota((8, 128), 1) & (128 - SB)) == a * SB for a in range(1, NS - 1)}
        zero = {r: jnp.zeros((r, 128), u32) for r in (8, 16)}
        slot = lambda n: _cols(n % NPS)

        def lane_select(pieces):
            keys = sorted(pieces)
            v = pieces[keys[0]]
            r = v.shape[0]
            for a in keys[1:]:
                v = lax.select(ge[r, a], pieces[a], v)
            if keys[0] > 0:
                v = lax.select(ge[r, keys[0]], v, zero[r])
            if keys[-1] < NS - 1:
                v = lax.select(ge[r, keys[-1] + 1], zero[r], v)
            return v

        def scores(n):
            qb, g, j = TILES[n]
            parts = [zero[8]] * 8
            for a in range(NS):
                hh = g * 8 + (j + a) % 8
                q = qt_ref[hh * 8:(hh + 1) * 8, _cols(qb)]
                parts[(j + a) % 8] = lax.select(eq[a], q, zero[8]) if a in eq else lane_select({a: q})
            ww = _as_bf16(jnp.concatenate(parts, axis=0))
            keys = lambda c0, c1: kw_ref[j % NS, (qb * 8 + c0) * 8:(qb * 8 + c1) * 8, _cols(g)]
            s0 = _dot(_as_bf16(jnp.concatenate(
                [keys(0, 1), keys(16, 17), keys(1, 2), keys(17, 18), keys(2, 3)], axis=0)), ww)
            rest = [_dot(_as_bf16(keys(c0, c1)), ww) for c0, c1 in ((3, 7), (7, 12), (12, 16))]
            first = lax.select(tri, jnp.concatenate([s0[0:16], s0[32:48]], axis=0),
                               jnp.concatenate([s0[16:32], s0[48:64]], axis=0))
            blocks = [jnp.concatenate([first, s0[64:80]], axis=0)] + rest
            p = jnp.exp2(jnp.concatenate(blocks, axis=0) - _col_max(blocks))
            pm = p[0:SB]
            p_ref.bitcast(bf16)[:, slot(n)] = jnp.concatenate(
                [lax.select(tri, pm, zero_p), p[SB:256], lax.select(tri, zero_p, pm)], axis=0).astype(bf16)
            return _col_sum(p)

        def pv(n):
            qb, g, j = TILES[n]
            src = [n - j + (j - a) % 8 for a in range(NS)]
            parts = []
            for t0, t1 in ((0, 2), (2, 4), (4, 6), (6, 18), (18, 20), (20, 22), (22, 24)):
                parts.append(lane_select(
                    {a: p_ref[(t0 - CB * a) * 8:(t1 - CB * a) * 8, slot(src[a])]
                     for a in range(NS) if 0 <= t0 - CB * a < NCH}))
            vt = vt_ref[(g * 8 + j) * 8:(g * 8 + j + 1) * 8, qb * 128:qb * 128 + 384]
            o = _dot(_as_bf16(vt), _as_bf16(jnp.concatenate(parts, axis=0)))
            l = lane_select({a: ls[src[a]] for a in range(NS)})
            heads.add(n, o * pl.reciprocal(l, approx=True))

        pv_at = {(n if n % 8 >= NS - 1 else n + 8): n for n in range(N)}
        heads, ls, fillers = _Heads(), {}, list(fillers)
        nq, npv, nf = 0, -4, -2
        while npv < N + 8:
            for tok in "QFQPP":
                if tok == "Q" and nq < N:
                    ls[nq] = scores(nq)
                    nq += 1
                elif tok == "P":
                    if npv == N - tail_pos:
                        tail()
                    if npv in pv_at:
                        pv(pv_at[npv])
                    npv += 1
                elif tok == "F":
                    if nf >= 0 and fillers:
                        fillers.pop(0)()
                    nf += 1
        assert not fillers
        return heads.result()

    def out_proj(t, o, mix=None):
        ys = []
        for r in range(0, TQ, 128):
            ob = o[r:r + 128].astype(bf16)
            if mix is None:
                ys.append(_dot(ob, wo_v[...]))
            else:
                cols = []
                for c in range(4):
                    cols.append(_dot(ob, wo_v[:, _cols(c)]))
                    for fl in mix.pop(0):
                        fl()
                ys.append(jnp.concatenate(cols, axis=1))
        x1 = x_v[rows_of(t), :].astype(f32) + modv(2) * jnp.concatenate(ys, axis=0)
        return x1, _modulate(_ln(x1), modv(4), modv(3))

    def h2_half(r):
        return _as_bf16(h2_ref[r * 64:(r + 1) * 64, :])

    last_copies = []

    def finish(t, c, x1, y):
        out = (x1 + mod_ref[0:1, _cols(20 + c)] * y).astype(bf16)
        if not (isinstance(t, int) and t == NTILES - 1):
            x_v[rows_of(t), _cols(c)] = out
            return
        nr = TQ // 4 if c == 3 else TQ
        for r in range(0, TQ, nr):
            idx = (slice(t * TQ + r, t * TQ + r + nr), _cols(c))
            x_v[idx] = out[r:r + nr]
            last_copies.append(pltpu.make_async_copy(x_v.at[idx], o_hbm.at[idx], sems.at[0]))
            last_copies[-1].start()

    def ffn1_tasks():
        def run(c, r):
            a_ref.bitcast(bf16)[r * 128:(r + 1) * 128, _cols(c)] = _silu(
                _dot(h2_half(r), w1_v[:, _cols(c)])).astype(bf16)
        return [functools.partial(run, c, r) for c in range(NFC) for r in range(2)]

    def ffn2(t, c):
        finish(t, c, x1_ref[:, _cols(c)], _dot(_as_bf16(a_ref[...]), w2_v[:, _cols(c)]))
        x1_ref[:, _cols(c)] = n_ref[0:TQ, _cols(c)]

    def ffn_value_tasks(get_h2, get_x1, t, early):
        acts, accs = {}, {}

        def run1(c, r):
            acts[(c, r)] = _silu(_dot(get_h2(r), w1_v[:, _cols(c)]))

        def run2(c, k0, k1):
            a = jnp.concatenate(
                [jnp.concatenate([acts[(k, r)] for k in range(k0, k1)], axis=1) for r in range(2)],
                axis=0).astype(bf16)
            y = _dot(a, w2_v[k0 * 128:k1 * 128, _cols(c)])
            if k0 > 0:
                y = y + accs.pop(c)
            if k1 < NFC:
                accs[c] = y
            else:
                finish(t, c, get_x1(c), y)

        t1 = [functools.partial(run1, c, r) for c in range(NFC) for r in range(2)]
        if not early:
            return t1, [functools.partial(run2, c, 0, NFC) for c in range(4)]
        for c in range(4):
            t1.insert(12 + c * 5, functools.partial(run2, c, 0, 4))
        return t1, [functools.partial(run2, c, 4, NFC) for c in range(4)]

    def mid_step(s, get_h, fill):
        def proj_q():
            qt_ref.bitcast(bf16)[...] = (t_dot(0, D, get_h()) * QSCALE).astype(bf16)
        o = attention(fill, proj_q, 1)
        advance_windows()
        x1, h2 = out_proj(s, o)
        h2_ref.bitcast(bf16)[...] = h2
        n_ref[0:TQ, :] = x1
        vt_ref[:, 0:TQ] = vt_ref[:, TQ:2 * TQ]
        vt_ref.bitcast(bf16)[:, TQ:2 * TQ] = t_dot(D, 2 * D, get_h()).astype(bf16)

    def once(fn):
        def body(i, carry):
            fn()
            return carry
        lax.fori_loop(1, cnt_ref[0], body, 0)

    cnt_ref[0] = 2
    d_c.wait()
    d_x01.wait()
    c = c_v[...].astype(f32)
    sc_ref[...] = jnp.broadcast_to(c * jax.nn.sigmoid(c), (16, D))
    n_ref[...] = _ln(x_v[0:2 * TQ, :].astype(f32))
    ha = lambda: _as_bf16(h01_ref[0:TQ // 2, :])
    hb = lambda: _as_bf16(h01_ref[TQ // 2:TQ, :])
    wt = wqvt_ref.bitcast(bf16)

    def h_cols(i):
        a, b = mparts[i]
        mod_cols(a, b)
        mod_cols(D + a, D + b)
        h01_ref.bitcast(bf16)[:, a:b] = _modulate(
            n_ref[:, a:b], mod_ref[0:1, D + a:D + b], mod_ref[0:1, a:b])

    for d in d_m[0]:
        d.wait()
    h_cols(0)
    for j in range(4):
        d_qk[j].wait()
        for d in (d_m[j] if j in (1, 2) else [d_wv] if j == 3 else []):
            d.wait()
        hj = _as_bf16(h01_ref[:, _cols(j)])
        ya = _dot(hj, wqkv_v[_cols(j), 0:D])
        if j in (1, 2):
            h_cols(j)
        y = jnp.concatenate([ya, _dot(hj, wqkv_v[_cols(j), D:2 * D])], axis=1)
        if j > 0:
            y = y + acc_ref[...]
        if j < 3:
            acc_ref[...] = y
        wt[0:D, _cols(j)] = wqkv_v[_cols(j), 0:D].astype(f32).T.astype(bf16)
    q0_ref.bitcast(bf16)[...] = (y[0:TQ, 0:D] * QSCALE).T.astype(bf16)
    qt_ref.bitcast(bf16)[...] = (y[TQ:2 * TQ, 0:D] * QSCALE).T.astype(bf16)
    k01_ref.bitcast(bf16)[...] = y[:, D:2 * D].astype(bf16)
    build_windows(k01_ref, 0, KW, alt=True)
    kp_ref[128:128 + KC, :] = k01_ref[TQ - KC:TQ, :]
    vt_ref.bitcast(bf16)[:, 0:TQ] = _dot(ha(), wqkv_v[:, 2 * D:3 * D]).T.astype(bf16)
    wt[D:2 * D, :] = wqkv_v[:, 2 * D:3 * D].astype(f32).T.astype(bf16)

    def v1(r, half):
        vt_ref.bitcast(bf16)[_cols(r), _cols(2 + half)] = t_dot(
            D + r * 128, D + (r + 1) * 128, hb()[_cols(half)]).astype(bf16)
    v1s = [functools.partial(v1, r, half) for r in range(4) for half in range(2)]
    o0 = attention_first(dict(zip((4, 2, 1, 0), v1s[:4])))
    d_wo.wait()
    d_mb.wait()
    d_x2.wait()

    def finish_tile0():
        m = [functools.partial(mod_cols, 2 * D + k * 128, 2 * D + (k + 1) * 128) for k in range(16)]
        h01_ref.bitcast(bf16)[0:TQ, :] = ln1(2)
        k = k_tasks(ha)
        x1, h2 = out_proj(0, o0, [
            m[0:2], m[2:4], m[4:5], [m[5], k[0], m[6], m[7], k[1], m[8], m[9], k[2], m[10], m[11]],
            m[12:13], m[13:14], m[14:15], [m[15], k[3]]])
        x1_ref[...] = x1
        h2_ref.bitcast(bf16)[...] = h2
    once(finish_tile0)

    d_w1.wait()
    once(lambda: mid_step(1, ha, v1s[4:] + ffn1_tasks()))
    d_w2.wait()
    d_xr.wait()

    def body(s, carry):
        ffn2(s - 2, 0)
        ffn2(s - 2, 1)
        h = ln1(s + 1)
        ffn2(s - 2, 2)
        ffn2(s - 2, 3)
        out_copy(s - 2).start()
        mid_step(s, lambda: h, ffn1_tasks() + k_tasks(lambda: h))
        return carry

    lax.fori_loop(2, NTILES - 1, body, 0)

    t = NTILES - 1
    for c in range(4):
        ffn2(t - 2, c)
    out_copy(t - 2).start()
    fill, rest = ffn_value_tasks(h2_half, lambda c: x1_ref[:, _cols(c)], t - 1, True)
    o = attention(fill, rest[0], -7)
    rest[1]()
    x1, h2 = out_proj(t, o)
    rest[2]()
    rest[3]()
    out_copy(t - 1).start()
    t1, t2 = ffn_value_tasks(lambda r: h2[_cols(r)], lambda c: x1[:, _cols(c)], t, False)
    for fl in t1 + t2:
        fl()
    for d in [out_copy(k) for k in range(NTILES - 1)] + last_copies:
        d.wait()


@jax.jit
def pallas_adaLN_cond__sliding_block__dense_activation_silu__prompt_kernel(
        A_x: jax.Array,
        A_wqkv: jax.Array,
        A_wo: jax.Array,
        B_x: jax.Array,
        B_w1: jax.Array,
        B_w2: jax.Array,
        c: jax.Array,
        w_mod: jax.Array,
):
    del B_x
    anyspec = pl.BlockSpec(memory_space=pl.ANY)
    out = pl.pallas_call(
        _kernel,
        in_specs=[anyspec] * 7,
        out_specs=anyspec,
        out_shape=jax.ShapeDtypeStruct((S, D), A_x.dtype),
        scratch_shapes=[
            pltpu.VMEM((S, D), bf16),
            pltpu.VMEM((D, 3 * D), bf16),
            pltpu.VMEM((D, D), bf16),
            pltpu.VMEM((D, F), bf16),
            pltpu.VMEM((F, D), bf16),
            pltpu.VMEM((1, D), bf16),
            pltpu.VMEM((D, 6 * D), bf16),
            pltpu.VMEM((8, 6 * D), f32),
            pltpu.VMEM((D, D), u32),
            pltpu.VMEM((D // 2, TQ), u32),
            pltpu.VMEM((D // 2, TQ), u32),
            pltpu.VMEM((KC + 128, D), u32),
            pltpu.VMEM((TQ, D), u32),
            pltpu.VMEM((NS, KW, D), u32),
            pltpu.VMEM((D // 2, 2 * TQ), u32),
            pltpu.VMEM((NCH * 8, NPS * 128), u32),
            pltpu.VMEM((TQ, D), f32),
            pltpu.VMEM((TQ // 2, D), u32),
            pltpu.VMEM((TQ, D), u32),
            pltpu.VMEM((2 * TQ, D), f32),
            pltpu.VMEM((2 * TQ, 2 * D), f32),
            pltpu.VMEM((TQ // 2, F), u32),
            pltpu.VMEM((16, D), f32),
            pltpu.SMEM((1,), jnp.int32),
            pltpu.SemaphoreType.DMA((9,)),
        ],
        compiler_params=pltpu.CompilerParams(vmem_limit_bytes=64 * 1024 * 1024),
    )(A_x.reshape(S, D), A_wqkv, A_wo, B_w1, B_w2, c, w_mod)
    return out.reshape(1, S, D)
```

```python
import functools

import jax
import jax.numpy as jnp
from jax import lax
import jax.experimental.pallas as pl
import jax.experimental.pallas.tpu as pltpu

S, D, DH, F = 2048, 512, 16, 1792
TQ = 256
NTILES = S // TQ
NFC = F // 128
EPS = 1e-5
QSCALE = (DH ** -0.5) * 1.4426950408889634
NEG = -1e30
NCH = 17
NPS = 32
bf16, u32, f32 = jnp.bfloat16, jnp.uint32, jnp.float32
NT_DIMS = (((1,), (1,)), ((), ()))
TILES = [(qb, g, j) for qb in range(TQ // 128) for g in range(4) for j in range(8)]
N = len(TILES)


def _iota(shape, dim):
    return lax.broadcasted_iota(jnp.int32, shape, dim)


def _ln(x):
    xc = x - jnp.mean(x, axis=-1, keepdims=True)
    ss = jnp.sum(xc * xc, axis=-1, keepdims=True) + D * EPS
    return xc * jnp.exp2(-0.5 * jnp.log2(ss))


def _modulate(n, scale, shift):
    return (n * ((1.0 + scale) * D ** 0.5) + shift).astype(bf16)


def _silu(z):
    hz = 0.5 * z
    return hz + hz * jnp.tanh(hz)


def _dot(a, b):
    return jnp.dot(a, b, preferred_element_type=f32)


def _as_bf16(x):
    return pltpu.bitcast(x, bf16)


def _cols(c):
    return slice(c * 128, (c + 1) * 128)


def _slot(n):
    return _cols(n % NPS)


def _col_max(blocks):
    ms = [functools.reduce(lax.max, [b[k:k + 8] for k in range(0, b.shape[0], 8)]) for b in blocks]
    while len(ms) > 1:
        ms = [lax.max(*ms[k:k + 2]) if k + 1 < len(ms) else ms[k] for k in range(0, len(ms), 2)]
    return jnp.max(ms[0], axis=0, keepdims=True)


def _col_sum(p):
    p = p.reshape(-1, 2, 2, 8, 128)
    v = jnp.sum(p[:, :, 0] + p[:, :, 1], axis=0)
    return jnp.sum(v[0] + v[1], axis=0, keepdims=True)


class _Lanes:
    def __init__(self, n):
        self.n, self.w = n, 128 // n
        w = self.w
        self.tri = _iota((w, 128), 0) > (_iota((w, 128), 1) & (w - 1))
        self.bit = {(r, k): (_iota((r, 128), 1) & (w << k)) != 0
                    for r in (1, w // 2, 64) for k in range(n.bit_length() - 1)}
        self.eq = [(_iota((8, 128), 1) & (128 - w)) == a * w for a in range(n)]
        self.zero = {r: jnp.zeros((r, 128), u32) for r in (8, w // 2)}

    def weights(self, q_ref, tile):
        qb, g, j = TILES[tile]
        a = j % self.n
        parts = [self.zero[8]] * 8
        for r in range(self.n):
            hh = g * 8 + j - a + r
            parts[hh % 8] = lax.select(self.eq[(a + r) % self.n],
                                       q_ref[hh * 8:(hh + 1) * 8, _cols(qb)], self.zero[8])
        return _as_bf16(jnp.concatenate(parts, axis=0))

    def unskew(self, xs, outs):
        n = self.n
        rows = next(x for x in xs if x is not None).shape[0]
        memo = {}

        def get(i, k):
            if k == 0:
                return xs[i % n]
            if (i % n, k) not in memo:
                lo, hi = get(i, k - 1), get(i + (1 << (k - 1)), k - 1)
                memo[i % n, k] = None if lo is None and hi is None else lax.select(
                    self.bit[rows, k - 1], self.zero[rows] if hi is None else hi,
                    self.zero[rows] if lo is None else lo)
            return memo[i % n, k]
        return [get(-r, n.bit_length() - 1) for r in outs]


class _Heads:
    def __init__(self, lanes, vt_ref, lazy_from=8):
        self.lanes, self.vt_ref, self.lazy_from = lanes, vt_ref, lazy_from
        self.ls, self.acc, self.ot, self.ob = {}, {}, {}, {}

    def pv(self, n0, outs, pieces, vcol, last):
        _, g, j0 = TILES[n0]
        cols = [self.lanes.unskew(xs, outs) for xs in pieces]
        for q, r in enumerate(outs):
            hh = g * 8 + j0 + r
            o = _dot(_as_bf16(self.vt_ref[hh * 8:(hh + 1) * 8, _cols(vcol)]),
                     _as_bf16(jnp.concatenate([c[q] for c in cols], axis=0)))
            self.acc[n0 + r] = o + self.acc[n0 + r] if n0 + r in self.acc else o
        if last:
            ls = self.lanes.unskew([self.ls[n0 + a] for a in range(self.lanes.n)], outs)
            for r, l in zip(outs, ls):
                k = n0 + r
                self.ot[k] = (self.acc.pop(k) * pl.reciprocal(l, approx=True), self.lanes.w * r)
                if k // 8 < self.lazy_from:
                    self._unrotate(k)
                    if all(kk in self.ot for kk in range(k // 8 * 8, k // 8 * 8 + 8)):
                        self._group(k // 8)

    def _unrotate(self, k):
        o, shift = self.ot[k]
        if shift:
            self.ot[k] = (pltpu.roll(o, 128 - shift, 1), 0)

    def _group(self, gi):
        if gi not in self.ob:
            ks = range(gi * 8, gi * 8 + 8)
            for k in ks:
                self._unrotate(k)
            self.ob[gi] = jnp.concatenate([self.ot[k][0] for k in ks], axis=0).T
        return self.ob[gi]

    def result(self):
        return jnp.concatenate(
            [jnp.concatenate([self._group(qb * 4 + g) for g in range(4)], axis=1)
             for qb in range(TQ // 128)], axis=0)


def _kernel(x_hbm, wqkv_hbm, wo_hbm, w1_hbm, w2_hbm, c_hbm, wmod_hbm, o_hbm,
            x_v, wqkv_v, wo_v, w1_v, w2_v, c_v, wmod_v,
            mod_ref, wqvt_ref, qt_ref, q0_ref, k_ref, vt_ref, p_ref,
            x1_ref, h2_ref, h01_ref, n_ref, acc_ref, a_ref, sc_ref, cnt_ref, sems):
    def cp(src, dst, idx, k):
        return pltpu.make_async_copy(src.at[idx], dst.at[idx], sems.at[k])
    al = slice(None)
    mparts = [(0, 256), (256, 384), (384, 512)]
    d_c = cp(c_hbm, c_v, (al, al), 0)
    d_x01 = cp(x_hbm, x_v, (slice(0, 2 * TQ), al), 0)
    d_m = [[cp(wmod_hbm, wmod_v, (al, slice(k * D + a, k * D + b)), (1, 3, 4)[i]) for k in range(2)]
           for i, (a, b) in enumerate(mparts)]
    d_qk = [cp(wqkv_hbm, wqkv_v, (_cols(j), slice(0, 2 * D)), 2 + j) for j in range(4)]
    d_wv = cp(wqkv_hbm, wqkv_v, (al, slice(2 * D, 3 * D)), 5)
    d_wo = cp(wo_hbm, wo_v, (al, al), 6)
    d_mb = cp(wmod_hbm, wmod_v, (al, slice(2 * D, 6 * D)), 6)
    d_x2 = cp(x_hbm, x_v, (slice(2 * TQ, 3 * TQ), al), 6)
    d_w1 = cp(w1_hbm, w1_v, (al, al), 7)
    d_w2 = cp(w2_hbm, w2_v, (al, al), 8)
    d_xr = cp(x_hbm, x_v, (slice(3 * TQ, S), al), 8)
    for d in ([d_c, d_x01] + d_m[0] + [d_qk[0]] + d_m[1] + [d_qk[1]] + d_m[2]
              + [d_qk[2], d_qk[3], d_wv, d_wo, d_mb, d_x2, d_w1, d_w2, d_xr]):
        d.start()

    def rows_of(t):
        return pl.ds(t * TQ if isinstance(t, int) else pl.multiple_of(t * TQ, TQ), TQ)

    def out_copy(t):
        return pltpu.make_async_copy(x_v.at[rows_of(t)], o_hbm.at[rows_of(t)], sems.at[0])

    def modv(k):
        return mod_ref[0:1, k * D:(k + 1) * D]

    def mod_cols(a, b):
        mod_ref[:, a:b] = _dot(sc_ref[...].astype(bf16), wmod_v[:, a:b])[0:8]

    def ln1(t):
        return _modulate(_ln(x_v[rows_of(t), :].astype(f32)), modv(1), modv(0))

    def k_tasks(get_h):
        def run(c):
            k_ref.bitcast(bf16)[2 * TQ:3 * TQ, _cols(c)] = _dot(
                get_h(), wqkv_v[:, _cols(4 + c)]).astype(bf16)
        return [functools.partial(run, c) for c in range(4)]

    def store_q(dst, qt, n):
        rows = []
        for hh in range(D // DH):
            q = qt[hh * DH:(hh + 1) * DH]
            if hh % n:
                q = jnp.concatenate(
                    [pltpu.roll(q[:, _cols(b)], 128 // n * (hh % n), 1) for b in range(2)], axis=1)
            rows.append(q)
        dst.bitcast(bf16)[...] = jnp.concatenate(rows, axis=0).astype(bf16)

    def t_dot(r0, r1, h):
        return lax.dot_general(_as_bf16(wqvt_ref[r0 // 2:r1 // 2, :]), h, NT_DIMS,
                               preferred_element_type=f32)

    def attention_first(fill):
        lanes = _Lanes(4)
        heads = _Heads(lanes, vt_ref, lazy_from=7)
        neg = jnp.full((32, 128), NEG, f32)

        def scores(n):
            qb, g, j = TILES[n]
            ww = lanes.weights(q0_ref, n)
            rows = qb * 128 + 32 * (j % 4 + 1)
            nsp = min(4, rows // 32)
            b = [(rows // 16 * k + nsp - 1) // nsp * 16 for k in range(nsp + 1)]
            s = jnp.concatenate([_dot(_as_bf16(k_ref[b[k] // 2:b[k + 1] // 2, _cols(g)]), ww)
                                 for k in range(nsp)], axis=0)
            last = lax.select(lanes.tri, neg, s[rows - 32:])
            s = jnp.concatenate([s[:rows - 32], last], axis=0) if rows > 32 else last
            p = jnp.exp2(s - _col_max([s[b[k]:b[k + 1]] for k in range(nsp)]))
            p_ref.bitcast(bf16)[0:rows, _slot(n)] = p.astype(bf16)
            heads.ls[n] = _col_sum(p)

        def pv(n0, k):
            qb = TILES[n0][0]
            if k < qb:
                pieces = [[p_ref[0:64, _slot(n0 + a)] for a in range(4)]]
            else:
                pieces = [[p_ref[qb * 64 + t * 16:qb * 64 + (t + 1) * 16, _slot(n0 + a)]
                           if a >= t else None for a in range(4)] for t in range(4)]
            heads.pv(n0, range(4), pieces, k, k == qb)

        due, at = {}, 0
        for n0 in range(0, N, 4):
            qb = TILES[n0][0]
            for k in range(qb + 1):
                at = max(at, n0 + (11, 9)[qb] + 2 * k)
                due.setdefault(at, []).append((n0, k))
        for i in range(at + 1):
            if i < N:
                scores(i - i % 4 + (2, 3, 1, 0)[i % 4])
            if i in fill:
                fill[i]()
            for step in due.get(i, []):
                pv(*step)
        return heads

    def attention(fillers, late):
        lanes = _Lanes(8)
        heads = _Heads(lanes, vt_ref)
        zero_p = jnp.zeros((16, 128), f32)

        def scores(n):
            qb, g, a = TILES[n]
            ww = lanes.weights(qt_ref, n)
            keys = lambda c0, c1: k_ref[(qb * 8 + a + c0) * 8:(qb * 8 + a + c1) * 8, _cols(g)]
            s = [_dot(_as_bf16(keys(c0, c1)), ww) for c0, c1 in ((1, 6), (6, 10), (10, 14))]
            e = _dot(_as_bf16(jnp.concatenate([keys(0, 1), keys(16, 17), keys(14, 16)], axis=0)), ww)
            edge = lax.select(lanes.tri, e[0:16], e[16:32])
            m = _col_max(s + [jnp.concatenate([edge, e[32:]], axis=0)])
            p = jnp.exp2(jnp.concatenate([edge] + s + [e[32:]], axis=0) - m)
            p_ref.bitcast(bf16)[:, _slot(n)] = jnp.concatenate(
                [lax.select(lanes.tri, p[0:16], zero_p), p[16:256],
                 lax.select(lanes.tri, zero_p, p[0:16])], axis=0).astype(bf16)
            heads.ls[n] = _col_sum(p)

        def pv(i):
            n0, k = i // 6 * 8, (1, 0, 2)[i % 3]
            rngs = [(8, 16)] if k == 1 else [(t, t + 1) for t in range(8 * k, 8 * k + 8)]
            pieces = [[p_ref[(t0 - a) * 8:(t1 - a) * 8, _slot(n0 + a)] if 0 <= t0 - a < NCH else None
                       for a in range(8)] for t0, t1 in rngs]
            heads.pv(n0, range(1 - i // 3 % 2, 8, 2), pieces, TILES[n0][0] + k, i % 3 == 2)

        fillers, late = list(fillers), list(late)
        nq, npv, nf = 0, -7, -3
        while npv < 48 or fillers or late:
            for tok in "QFQPQFQPP":
                if tok == "Q" and nq < N:
                    scores(nq)
                    nq += 1
                elif tok == "P":
                    if 0 <= npv < 48:
                        pv(npv)
                    npv += 1
                elif tok == "F":
                    if nf >= 0 and fillers:
                        fillers.pop(0)()
                    elif nq >= N and late:
                        late.pop(0)()
                    nf += 1
        return heads.result()

    def out_proj(t, o, mix=None):
        ys = []
        for r in range(0, TQ, 128):
            ob = o[r:r + 128].astype(bf16)
            if mix is None:
                ys.append(_dot(ob, wo_v[...]))
            else:
                cols = []
                for c in range(4):
                    cols.append(_dot(ob, wo_v[:, _cols(c)]))
                    for fl in mix.pop(0):
                        fl()
                ys.append(jnp.concatenate(cols, axis=1))
        x1 = x_v[rows_of(t), :].astype(f32) + modv(2) * jnp.concatenate(ys, axis=0)
        return x1, _modulate(_ln(x1), modv(4), modv(3))

    def h2_half(r):
        return _as_bf16(h2_ref[r * 64:(r + 1) * 64, :])

    last_copies = []

    def finish(t, c, x1, y):
        out = (x1 + mod_ref[0:1, _cols(20 + c)] * y).astype(bf16)
        if not (isinstance(t, int) and t == NTILES - 1):
            x_v[rows_of(t), _cols(c)] = out
            return
        nr = TQ // 4 if c == 3 else TQ
        for r in range(0, TQ, nr):
            idx = (slice(t * TQ + r, t * TQ + r + nr), _cols(c))
            x_v[idx] = out[r:r + nr]
            last_copies.append(pltpu.make_async_copy(x_v.at[idx], o_hbm.at[idx], sems.at[0]))
            last_copies[-1].start()

    def ffn1_tasks():
        def run(c, r):
            a_ref.bitcast(bf16)[r * 128:(r + 1) * 128, _cols(c)] = _silu(
                _dot(h2_half(r), w1_v[:, _cols(c)])).astype(bf16)
        return [functools.partial(run, c, r) for c in range(NFC) for r in range(2)]

    def ffn2(t, c):
        finish(t, c, x1_ref[:, _cols(c)], _dot(_as_bf16(a_ref[...]), w2_v[:, _cols(c)]))
        x1_ref[:, _cols(c)] = n_ref[0:TQ, _cols(c)]

    def ffn_value_tasks(get_h2, get_x1, t, split):
        acts, accs = {}, {}

        def run1(c, r):
            acts[(c, r)] = _silu(_dot(get_h2(r), w1_v[:, _cols(c)]))

        def run2(c, k0, k1):
            a = jnp.concatenate(
                [jnp.concatenate([acts[(k, r)] for k in range(k0, k1)], axis=1) for r in range(2)],
                axis=0).astype(bf16)
            y = _dot(a, w2_v[k0 * 128:k1 * 128, _cols(c)])
            if k0 > 0:
                y = y + accs.pop(c)
            if k1 < NFC:
                accs[c] = y
            else:
                finish(t, c, get_x1(c), y)

        t1 = [functools.partial(run1, c, r) for c in range(NFC) for r in range(2)]
        if not split:
            return t1, [functools.partial(run2, c, 0, NFC) for c in range(4)]
        return (t1 + [functools.partial(run2, c, 0, 4) for c in range(4)],
                [functools.partial(run2, c, 4, NFC) for c in range(4)])

    def mid_step(s, get_h, fill):
        o = attention(fill, [lambda: store_q(qt_ref, t_dot(0, D, get_h()) * QSCALE, 8)])
        k_ref[0:TQ // 2, :] = k_ref[TQ // 2:TQ, :]
        k_ref[TQ // 2:TQ, :] = k_ref[TQ:3 * TQ // 2, :]
        x1, h2 = out_proj(s, o)
        h2_ref.bitcast(bf16)[...] = h2
        n_ref[0:TQ, :] = x1
        vt_ref[:, 0:TQ] = vt_ref[:, TQ:2 * TQ]
        vt_ref.bitcast(bf16)[:, TQ:2 * TQ] = t_dot(D, 2 * D, get_h()).astype(bf16)

    def once(fn):
        def body(i, carry):
            fn()
            return carry
        lax.fori_loop(1, cnt_ref[0], body, 0)

    cnt_ref[0] = 2
    d_c.wait()
    d_x01.wait()
    c = c_v[...].astype(f32)
    sc_ref[...] = jnp.broadcast_to(c * jax.nn.sigmoid(c), (16, D))
    n_ref[...] = _ln(x_v[0:2 * TQ, :].astype(f32))
    ha = lambda: _as_bf16(h01_ref[0:TQ // 2, :])
    hb = lambda: _as_bf16(h01_ref[TQ // 2:TQ, :])
    wt = wqvt_ref.bitcast(bf16)

    def h_cols(i):
        a, b = mparts[i]
        mod_cols(a, b)
        mod_cols(D + a, D + b)
        h01_ref.bitcast(bf16)[:, a:b] = _modulate(
            n_ref[:, a:b], mod_ref[0:1, D + a:D + b], mod_ref[0:1, a:b])

    for d in d_m[0]:
        d.wait()
    h_cols(0)
    for j in range(4):
        d_qk[j].wait()
        for d in (d_m[j] if j in (1, 2) else [d_wv] if j == 3 else []):
            d.wait()
        hj = _as_bf16(h01_ref[:, _cols(j)])
        ya = _dot(hj, wqkv_v[_cols(j), 0:D])
        if j in (1, 2):
            h_cols(j)
        y = jnp.concatenate([ya, _dot(hj, wqkv_v[_cols(j), D:2 * D])], axis=1)
        if j > 0:
            y = y + acc_ref[...]
        if j < 3:
            acc_ref[...] = y
        wt[0:D, _cols(j)] = wqkv_v[_cols(j), 0:D].astype(f32).T.astype(bf16)
    store_q(q0_ref, (y[0:TQ, 0:D] * QSCALE).T, 4)
    store_q(qt_ref, (y[TQ:2 * TQ, 0:D] * QSCALE).T, 8)
    k_ref.bitcast(bf16)[0:2 * TQ, :] = y[:, D:2 * D].astype(bf16)
    wt[D:2 * D, :] = wqkv_v[:, 2 * D:3 * D].astype(f32).T.astype(bf16)
    vt_ref.bitcast(bf16)[:, 0:TQ] = t_dot(D, 2 * D, ha()).astype(bf16)

    def v1(r, half):
        vt_ref.bitcast(bf16)[_cols(r), _cols(2 + half)] = t_dot(
            D + r * 128, D + (r + 1) * 128, hb()[_cols(half)]).astype(bf16)
    heads0 = attention_first(dict(zip(
        (3, 11, 12, 18, 40, 64, 66, 68),
        [functools.partial(v1, r, half) for r in range(4) for half in range(2)])))
    d_wo.wait()
    d_mb.wait()
    d_x2.wait()

    def finish_tile0():
        m = [functools.partial(mod_cols, 2 * D + k * 128, 2 * D + (k + 1) * 128) for k in range(16)]
        h01_ref.bitcast(bf16)[0:TQ, :] = ln1(2)
        k = k_tasks(ha)
        x1, h2 = out_proj(0, heads0.result(), [
            m[0:2], m[2:4], m[4:5], [m[5], k[0], m[6], m[7], k[1], m[8], m[9], k[2], m[10], m[11]],
            m[12:13], m[13:14], m[14:15], [m[15], k[3]]])
        x1_ref[...] = x1
        h2_ref.bitcast(bf16)[...] = h2
    once(finish_tile0)

    d_w1.wait()
    once(lambda: mid_step(1, ha, ffn1_tasks()))
    d_w2.wait()
    d_xr.wait()

    def body(s, carry):
        ffn2(s - 2, 0)
        ffn2(s - 2, 1)
        h = ln1(s + 1)
        ffn2(s - 2, 2)
        ffn2(s - 2, 3)
        out_copy(s - 2).start()
        mid_step(s, lambda: h, ffn1_tasks() + k_tasks(lambda: h))
        return carry

    lax.fori_loop(2, NTILES - 1, body, 0)

    t = NTILES - 1
    for c in range(4):
        ffn2(t - 2, c)
    out_copy(t - 2).start()
    fill, rest = ffn_value_tasks(h2_half, lambda c: x1_ref[:, _cols(c)], t - 1, True)
    o = attention(fill, [])
    rest[0]()
    rest[1]()
    x1, h2 = out_proj(t, o)
    rest[2]()
    rest[3]()
    out_copy(t - 1).start()
    t1, t2 = ffn_value_tasks(lambda r: h2[_cols(r)], lambda c: x1[:, _cols(c)], t, False)
    for fl in t1 + t2:
        fl()
    for d in [out_copy(k) for k in range(NTILES - 1)] + last_copies:
        d.wait()


@jax.jit
def pallas_adaLN_cond__sliding_block__dense_activation_silu__prompt_kernel(
        A_x: jax.Array,
        A_wqkv: jax.Array,
        A_wo: jax.Array,
        B_x: jax.Array,
        B_w1: jax.Array,
        B_w2: jax.Array,
        c: jax.Array,
        w_mod: jax.Array,
):
    del B_x
    anyspec = pl.BlockSpec(memory_space=pl.ANY)
    out = pl.pallas_call(
        _kernel,
        in_specs=[anyspec] * 7,
        out_specs=anyspec,
        out_shape=jax.ShapeDtypeStruct((S, D), A_x.dtype),
        scratch_shapes=[
            pltpu.VMEM((S, D), bf16),
            pltpu.VMEM((D, 3 * D), bf16),
            pltpu.VMEM((D, D), bf16),
            pltpu.VMEM((D, F), bf16),
            pltpu.VMEM((F, D), bf16),
            pltpu.VMEM((1, D), bf16),
            pltpu.VMEM((D, 6 * D), bf16),
            pltpu.VMEM((8, 6 * D), f32),
            pltpu.VMEM((D, D), u32),
            pltpu.VMEM((D // 2, TQ), u32),
            pltpu.VMEM((D // 2, TQ), u32),
            pltpu.VMEM((3 * TQ // 2, D), u32),
            pltpu.VMEM((D // 2, 2 * TQ), u32),
            pltpu.VMEM((NCH * 8, NPS * 128), u32),
            pltpu.VMEM((TQ, D), f32),
            pltpu.VMEM((TQ // 2, D), u32),
            pltpu.VMEM((TQ, D), u32),
            pltpu.VMEM((2 * TQ, D), f32),
            pltpu.VMEM((2 * TQ, 2 * D), f32),
            pltpu.VMEM((TQ // 2, F), u32),
            pltpu.VMEM((16, D), f32),
            pltpu.SMEM((1,), jnp.int32),
            pltpu.SemaphoreType.DMA((9,)),
        ],
        compiler_params=pltpu.CompilerParams(vmem_limit_bytes=64 * 1024 * 1024),
    )(A_x.reshape(S, D), A_wqkv, A_wo, B_w1, B_w2, c, w_mod)
    return out.reshape(1, S, D)
```

```python
import functools

import jax
import jax.numpy as jnp
from jax import lax
import jax.experimental.pallas as pl
import jax.experimental.pallas.tpu as pltpu

S, D, DH, F = 2048, 512, 16, 1792
TQ = 256
NTILES = S // TQ
NFC = F // 128
EPS = 1e-5
QSCALE = (DH ** -0.5) * 1.4426950408889634
NEG = -1e30
NCH = 17
NPS = 32
bf16, u32, f32 = jnp.bfloat16, jnp.uint32, jnp.float32
NT_DIMS = (((1,), (1,)), ((), ()))
TILES = [(qb, g, j) for qb in range(TQ // 128) for g in range(4) for j in range(8)]
N = len(TILES)


def _iota(shape, dim):
    return lax.broadcasted_iota(jnp.int32, shape, dim)


def _ln(x):
    xc = x - jnp.mean(x, axis=-1, keepdims=True)
    ss = jnp.sum(xc * xc, axis=-1, keepdims=True) + D * EPS
    return xc * jnp.exp2(-0.5 * jnp.log2(ss))


def _modulate(n, scale, shift):
    return (n * ((1.0 + scale) * D ** 0.5) + shift).astype(bf16)


def _silu(z):
    hz = 0.5 * z
    return hz + hz * jnp.tanh(hz)


def _dot(a, b):
    return jnp.dot(a, b, preferred_element_type=f32)


def _as_bf16(x):
    return pltpu.bitcast(x, bf16)


def _cols(c):
    return slice(c * 128, (c + 1) * 128)


def _slot(n):
    return _cols(n % NPS)


def _col_max(blocks):
    ms = [functools.reduce(lax.max, [b[k:k + 8] for k in range(0, b.shape[0], 8)]) for b in blocks]
    while len(ms) > 1:
        ms = [lax.max(*ms[k:k + 2]) if k + 1 < len(ms) else ms[k] for k in range(0, len(ms), 2)]
    return jnp.max(ms[0], axis=0, keepdims=True)


def _col_sum(p):
    p = p.reshape(-1, 2, 2, 8, 128)
    v = jnp.sum(p[:, :, 0] + p[:, :, 1], axis=0)
    return jnp.sum(v[0] + v[1], axis=0, keepdims=True)


class _Lanes:
    def __init__(self, n):
        self.n, self.w = n, 128 // n
        w = self.w
        self.tri = _iota((w, 128), 0) > (_iota((w, 128), 1) & (w - 1))
        self.bit = {(r, k): (_iota((r, 128), 1) & (w << k)) != 0
                    for r in (1, w // 2, 64) for k in range(n.bit_length() - 1)}
        self.eq = [(_iota((8, 128), 1) & (128 - w)) == a * w for a in range(n)]
        self.zero = {r: jnp.zeros((r, 128), u32) for r in (8, w // 2)}

    def weights(self, q_ref, tile):
        qb, g, j = TILES[tile]
        a = j % self.n
        parts = [self.zero[8]] * 8
        for r in range(self.n):
            hh = g * 8 + j - a + r
            parts[hh % 8] = lax.select(self.eq[(a + r) % self.n],
                                       q_ref[hh * 8:(hh + 1) * 8, _cols(qb)], self.zero[8])
        return _as_bf16(jnp.concatenate(parts, axis=0))

    def unskew(self, xs, outs):
        n = self.n
        rows = next(x for x in xs if x is not None).shape[0]
        memo = {}

        def get(i, k):
            if k == 0:
                return xs[i % n]
            if (i % n, k) not in memo:
                lo, hi = get(i, k - 1), get(i + (1 << (k - 1)), k - 1)
                memo[i % n, k] = None if lo is None and hi is None else lax.select(
                    self.bit[rows, k - 1], self.zero[rows] if hi is None else hi,
                    self.zero[rows] if lo is None else lo)
            return memo[i % n, k]
        return [get(-r, n.bit_length() - 1) for r in outs]


class _Heads:
    def __init__(self, lanes, vt_ref, lazy_from=8):
        self.lanes, self.vt_ref, self.lazy_from = lanes, vt_ref, lazy_from
        self.ls, self.acc, self.ot, self.ob = {}, {}, {}, {}

    def pv(self, n0, outs, pieces, vcol, last):
        _, g, j0 = TILES[n0]
        cols = [self.lanes.unskew(xs, outs) for xs in pieces]
        for q, r in enumerate(outs):
            hh = g * 8 + j0 + r
            o = _dot(_as_bf16(self.vt_ref[hh * 8:(hh + 1) * 8, _cols(vcol)]),
                     _as_bf16(jnp.concatenate([c[q] for c in cols], axis=0)))
            self.acc[n0 + r] = o + self.acc[n0 + r] if n0 + r in self.acc else o
        if last:
            ls = self.lanes.unskew([self.ls[n0 + a] for a in range(self.lanes.n)], outs)
            for r, l in zip(outs, ls):
                k = n0 + r
                self.ot[k] = (self.acc.pop(k) * pl.reciprocal(l, approx=True), self.lanes.w * r)
                if k // 8 < self.lazy_from:
                    self._unrotate(k)
                    if all(kk in self.ot for kk in range(k // 8 * 8, k // 8 * 8 + 8)):
                        self._group(k // 8)

    def _unrotate(self, k):
        o, shift = self.ot[k]
        if shift:
            self.ot[k] = (pltpu.roll(o, 128 - shift, 1), 0)

    def _group(self, gi):
        if gi not in self.ob:
            ks = range(gi * 8, gi * 8 + 8)
            for k in ks:
                self._unrotate(k)
            self.ob[gi] = jnp.concatenate([self.ot[k][0] for k in ks], axis=0).T
        return self.ob[gi]

    def result(self):
        return jnp.concatenate(
            [jnp.concatenate([self._group(qb * 4 + g) for g in range(4)], axis=1)
             for qb in range(TQ // 128)], axis=0)


def _kernel(x_hbm, wqkv_hbm, wo_hbm, w1_hbm, w2_hbm, c_hbm, wmod_hbm, o_hbm,
            x_v, wqkv_v, wo_v, w1_v, w2_v, c_v, wmod_v,
            mod_ref, wqvt_ref, qt_ref, q0_ref, k_ref, vt_ref, p_ref,
            x1_ref, h2_ref, h01_ref, n_ref, acc_ref, a_ref, sc_ref, cnt_ref, sems):
    def cp(src, dst, idx, k):
        return pltpu.make_async_copy(src.at[idx], dst.at[idx], sems.at[k])
    al = slice(None)
    mparts = [(0, 256), (256, 384), (384, 512)]
    d_c = cp(c_hbm, c_v, (al, al), 0)
    d_x01 = cp(x_hbm, x_v, (slice(0, 2 * TQ), al), 0)
    d_m = [[cp(wmod_hbm, wmod_v, (al, slice(k * D + a, k * D + b)), (1, 3, 4)[i]) for k in range(2)]
           for i, (a, b) in enumerate(mparts)]
    d_qk = [cp(wqkv_hbm, wqkv_v, (_cols(j), slice(0, 2 * D)), 2 + j) for j in range(4)]
    d_wv = cp(wqkv_hbm, wqkv_v, (al, slice(2 * D, 3 * D)), 5)
    d_wo = cp(wo_hbm, wo_v, (al, al), 6)
    d_mb = cp(wmod_hbm, wmod_v, (al, slice(2 * D, 6 * D)), 6)
    d_x2 = cp(x_hbm, x_v, (slice(2 * TQ, 3 * TQ), al), 6)
    d_w1 = cp(w1_hbm, w1_v, (al, al), 7)
    d_w2 = cp(w2_hbm, w2_v, (al, al), 8)
    d_xr = cp(x_hbm, x_v, (slice(3 * TQ, S), al), 8)
    for d in ([d_c, d_x01] + d_m[0] + [d_qk[0]] + d_m[1] + [d_qk[1]] + d_m[2]
              + [d_qk[2], d_qk[3], d_wv, d_wo, d_mb, d_x2, d_w1, d_w2, d_xr]):
        d.start()

    def rows_of(t):
        return pl.ds(t * TQ if isinstance(t, int) else pl.multiple_of(t * TQ, TQ), TQ)

    def out_copy(t):
        return pltpu.make_async_copy(x_v.at[rows_of(t)], o_hbm.at[rows_of(t)], sems.at[0])

    def modv(k):
        return mod_ref[0:1, k * D:(k + 1) * D]

    def mod_cols(a, b):
        mod_ref[:, a:b] = _dot(sc_ref[...].astype(bf16), wmod_v[:, a:b])[0:8]

    def ln1(t):
        return _modulate(_ln(x_v[rows_of(t), :].astype(f32)), modv(1), modv(0))

    def k_tasks(get_h):
        def run(c):
            k_ref.bitcast(bf16)[2 * TQ:3 * TQ, _cols(c)] = _dot(
                get_h(), wqkv_v[:, _cols(4 + c)]).astype(bf16)
        return [functools.partial(run, c) for c in range(4)]

    def store_q(dst, qt, n):
        rows = []
        for hh in range(D // DH):
            q = qt[hh * DH:(hh + 1) * DH]
            if hh % n:
                q = jnp.concatenate(
                    [pltpu.roll(q[:, _cols(b)], 128 // n * (hh % n), 1) for b in range(2)], axis=1)
            rows.append(q)
        dst.bitcast(bf16)[...] = jnp.concatenate(rows, axis=0).astype(bf16)

    def t_dot(r0, r1, h):
        return lax.dot_general(_as_bf16(wqvt_ref[r0 // 2:r1 // 2, :]), h, NT_DIMS,
                               preferred_element_type=f32)

    def attention_first(fill):
        lanes = _Lanes(4)
        heads = _Heads(lanes, vt_ref, lazy_from=7)
        neg = jnp.full((32, 128), NEG, f32)

        def scores(n):
            qb, g, j = TILES[n]
            ww = lanes.weights(q0_ref, n)
            rows = qb * 128 + 32 * (j % 4 + 1)
            nsp = min(4, rows // 32)
            b = [(rows // 16 * k + nsp - 1) // nsp * 16 for k in range(nsp + 1)]
            s = jnp.concatenate([_dot(_as_bf16(k_ref[b[k] // 2:b[k + 1] // 2, _cols(g)]), ww)
                                 for k in range(nsp)], axis=0)
            last = lax.select(lanes.tri, neg, s[rows - 32:])
            s = jnp.concatenate([s[:rows - 32], last], axis=0) if rows > 32 else last
            p = jnp.exp2(s - _col_max([s[b[k]:b[k + 1]] for k in range(nsp)]))
            p_ref.bitcast(bf16)[0:rows, _slot(n)] = p.astype(bf16)
            heads.ls[n] = _col_sum(p)

        def pv(n0, k):
            qb = TILES[n0][0]
            if k < qb:
                pieces = [[p_ref[0:64, _slot(n0 + a)] for a in range(4)]]
            else:
                pieces = [[p_ref[qb * 64 + t * 16:qb * 64 + (t + 1) * 16, _slot(n0 + a)]
                           if a >= t else None for a in range(4)] for t in range(4)]
            heads.pv(n0, range(4), pieces, k, k == qb)

        due, at = {}, 0
        for n0 in range(0, N, 4):
            qb = TILES[n0][0]
            for k in range(qb + 1):
                at = max(at, n0 + (11, 9)[qb] + 2 * k)
                due.setdefault(at, []).append((n0, k))
        for i in range(at + 1):
            if i < N:
                scores(i - i % 4 + (2, 3, 1, 0)[i % 4])
            if i in fill:
                fill[i]()
            for step in due.get(i, []):
                pv(*step)
        return heads

    def attention(fillers, late, head=(), skip=3):
        lanes = _Lanes(8)
        heads = _Heads(lanes, vt_ref)
        zero_p = jnp.zeros((16, 128), f32)

        def scores(n):
            qb, g, a = TILES[n]
            ww = lanes.weights(qt_ref, n)
            keys = lambda c0, c1: k_ref[(qb * 8 + a + c0) * 8:(qb * 8 + a + c1) * 8, _cols(g)]
            s = [_dot(_as_bf16(keys(c0, c1)), ww) for c0, c1 in ((1, 6), (6, 10), (10, 14))]
            e = _dot(_as_bf16(jnp.concatenate([keys(0, 1), keys(16, 17), keys(14, 16)], axis=0)), ww)
            edge = lax.select(lanes.tri, e[0:16], e[16:32])
            m = _col_max(s + [jnp.concatenate([edge, e[32:]], axis=0)])
            p = jnp.exp2(jnp.concatenate([edge] + s + [e[32:]], axis=0) - m)
            p_ref.bitcast(bf16)[:, _slot(n)] = jnp.concatenate(
                [lax.select(lanes.tri, p[0:16], zero_p), p[16:256],
                 lax.select(lanes.tri, zero_p, p[0:16])], axis=0).astype(bf16)
            heads.ls[n] = _col_sum(p)

        def pv(i):
            n0, k = i // 6 * 8, (1, 0, 2)[i % 3]
            rngs = [(8, 16)] if k == 1 else [(t, t + 1) for t in range(8 * k, 8 * k + 8)]
            pieces = [[p_ref[(t0 - a) * 8:(t1 - a) * 8, _slot(n0 + a)] if 0 <= t0 - a < NCH else None
                       for a in range(8)] for t0, t1 in rngs]
            heads.pv(n0, range(1 - i // 3 % 2, 8, 2), pieces, TILES[n0][0] + k, i % 3 == 2)

        fillers, late, nq = list(fillers), list(late), 0
        for fl in head:
            if fl is None:
                scores(nq)
                nq += 1
            else:
                fl()
        npv, nf = -7 + 3 * nq // 4, -skip
        while npv < 48 or fillers or late:
            for tok in "QFQPQFQPP":
                if tok == "Q" and nq < N:
                    scores(nq)
                    nq += 1
                elif tok == "P":
                    if 0 <= npv < 48:
                        pv(npv)
                    npv += 1
                elif tok == "F":
                    if nf >= 0 and fillers:
                        fillers.pop(0)()
                    elif nq >= N and late:
                        late.pop(0)()
                    nf += 1
        return heads.result()

    def out_proj(t, o, mix=None):
        ys = []
        for r in range(0, TQ, 128):
            ob = o[r:r + 128].astype(bf16)
            if mix is None:
                ys.append(_dot(ob, wo_v[...]))
            else:
                cols = []
                for c in range(4):
                    cols.append(_dot(ob, wo_v[:, _cols(c)]))
                    for fl in mix.pop(0):
                        fl()
                ys.append(jnp.concatenate(cols, axis=1))
        x1 = x_v[rows_of(t), :].astype(f32) + modv(2) * jnp.concatenate(ys, axis=0)
        return x1, _modulate(_ln(x1), modv(4), modv(3))

    def h2_half(r):
        return _as_bf16(h2_ref[r * 64:(r + 1) * 64, :])

    last_copies = []

    def finish(t, c, x1, y):
        out = (x1 + mod_ref[0:1, _cols(20 + c)] * y).astype(bf16)
        if not (isinstance(t, int) and t == NTILES - 1):
            x_v[rows_of(t), _cols(c)] = out
            return
        nr = TQ // 4 if c == 3 else TQ
        for r in range(0, TQ, nr):
            idx = (slice(t * TQ + r, t * TQ + r + nr), _cols(c))
            x_v[idx] = out[r:r + nr]
            last_copies.append(pltpu.make_async_copy(x_v.at[idx], o_hbm.at[idx], sems.at[0]))
            last_copies[-1].start()

    def ffn1_tasks():
        def run(c, r):
            a_ref.bitcast(bf16)[r * 128:(r + 1) * 128, _cols(c)] = _silu(
                _dot(h2_half(r), w1_v[:, _cols(c)])).astype(bf16)
        return [functools.partial(run, c, r) for c in range(NFC) for r in range(2)]

    def ffn2(t, cs):
        for c in cs:
            finish(t, c, x1_ref[:, _cols(c)], _dot(_as_bf16(a_ref[...]), w2_v[:, _cols(c)]))
            x1_ref[:, _cols(c)] = n_ref[0:TQ, _cols(c)]
        if c == 3:
            out_copy(t).start()

    def ffn_value_tasks(get_h2, get_x1, t, split):
        acts, accs = {}, {}

        def run1(c, r):
            acts[(c, r)] = _silu(_dot(get_h2(r), w1_v[:, _cols(c)]))

        def run2(c, k0, k1):
            a = jnp.concatenate(
                [jnp.concatenate([acts[(k, r)] for k in range(k0, k1)], axis=1) for r in range(2)],
                axis=0).astype(bf16)
            y = _dot(a, w2_v[k0 * 128:k1 * 128, _cols(c)])
            if k0 > 0:
                y = y + accs.pop(c)
            if k1 < NFC:
                accs[c] = y
            else:
                finish(t, c, get_x1(c), y)

        t1 = [functools.partial(run1, c, r) for c in range(NFC) for r in range(2)]
        if not split:
            return t1, [functools.partial(run2, c, 0, NFC) for c in range(4)]
        return (t1 + [functools.partial(run2, c, 0, 8) for c in range(4)],
                [functools.partial(run2, c, 8, NFC) for c in range(4)])

    def mid_step(s, get_h, fill, *order):
        o = attention(fill, [lambda: store_q(qt_ref, t_dot(0, D, get_h()) * QSCALE, 8)], *order)
        k_ref[0:TQ // 2, :] = k_ref[TQ // 2:TQ, :]
        k_ref[TQ // 2:TQ, :] = k_ref[TQ:3 * TQ // 2, :]
        x1, h2 = out_proj(s, o)
        h2_ref.bitcast(bf16)[...] = h2
        n_ref[0:TQ, :] = x1
        vt_ref[:, 0:TQ] = vt_ref[:, TQ:2 * TQ]
        vt_ref.bitcast(bf16)[:, TQ:2 * TQ] = t_dot(D, 2 * D, get_h()).astype(bf16)

    def once(fn):
        def body(i, carry):
            fn()
            return carry
        lax.fori_loop(1, cnt_ref[0], body, 0)

    cnt_ref[0] = 2
    d_c.wait()
    d_x01.wait()
    c = c_v[...].astype(f32)
    sc_ref[...] = jnp.broadcast_to(c * jax.nn.sigmoid(c), (16, D))
    n_ref[...] = _ln(x_v[0:2 * TQ, :].astype(f32))
    ha = lambda: _as_bf16(h01_ref[0:TQ // 2, :])
    hb = lambda: _as_bf16(h01_ref[TQ // 2:TQ, :])
    wt = wqvt_ref.bitcast(bf16)

    def h_cols(i):
        a, b = mparts[i]
        mod_cols(a, b)
        mod_cols(D + a, D + b)
        h01_ref.bitcast(bf16)[:, a:b] = _modulate(
            n_ref[:, a:b], mod_ref[0:1, D + a:D + b], mod_ref[0:1, a:b])

    for d in d_m[0]:
        d.wait()
    h_cols(0)
    for j in range(4):
        d_qk[j].wait()
        for d in (d_m[j] if j in (1, 2) else [d_wv] if j == 3 else []):
            d.wait()
        hj = _as_bf16(h01_ref[:, _cols(j)])
        ya = _dot(hj, wqkv_v[_cols(j), 0:D])
        if j in (1, 2):
            h_cols(j)
        y = jnp.concatenate([ya, _dot(hj, wqkv_v[_cols(j), D:2 * D])], axis=1)
        if j > 0:
            y = y + acc_ref[...]
        if j < 3:
            acc_ref[...] = y
        wt[0:D, _cols(j)] = wqkv_v[_cols(j), 0:D].astype(f32).T.astype(bf16)
    store_q(q0_ref, (y[0:TQ, 0:D] * QSCALE).T, 4)
    store_q(qt_ref, (y[TQ:2 * TQ, 0:D] * QSCALE).T, 8)
    k_ref.bitcast(bf16)[0:2 * TQ, :] = y[:, D:2 * D].astype(bf16)
    wt[D:2 * D, :] = wqkv_v[:, 2 * D:3 * D].astype(f32).T.astype(bf16)
    vt_ref.bitcast(bf16)[:, 0:TQ] = t_dot(D, 2 * D, ha()).astype(bf16)

    def v1(r, half):
        vt_ref.bitcast(bf16)[_cols(r), _cols(2 + half)] = t_dot(
            D + r * 128, D + (r + 1) * 128, hb()[_cols(half)]).astype(bf16)
    heads0 = attention_first(dict(zip(
        (3, 11, 12, 18, 40, 64, 66, 68),
        [functools.partial(v1, r, half) for r in range(4) for half in range(2)])))
    d_wo.wait()
    d_mb.wait()
    d_x2.wait()

    def finish_tile0():
        m = [functools.partial(mod_cols, 2 * D + k * 128, 2 * D + (k + 1) * 128) for k in range(16)]
        h01_ref.bitcast(bf16)[0:TQ, :] = ln1(2)
        k = k_tasks(ha)
        x1, h2 = out_proj(0, heads0.result(), [
            m[0:2], m[2:4], m[4:5], [m[5], k[0], m[6], m[7], k[1], m[8], m[9], k[2], m[10], m[11]],
            m[12:13], m[13:14], m[14:15], [m[15], k[3]]])
        x1_ref[...] = x1
        h2_ref.bitcast(bf16)[...] = h2
    once(finish_tile0)

    d_w1.wait()
    once(lambda: mid_step(1, ha, ffn1_tasks()))
    d_w2.wait()
    d_xr.wait()

    def body(s, carry):
        h = []

        def finish_old():
            ffn2(s - 2, (0, 1))
            h.append(ln1(s + 1))
            ffn2(s - 2, (2, 3))
        mid_step(s, lambda: h[0], ffn1_tasks() + k_tasks(lambda: h[0]), [None] * 8 + [finish_old], 1)
        return carry

    lax.fori_loop(2, NTILES - 1, body, 0)

    t = NTILES - 1
    fill, rest = ffn_value_tasks(h2_half, lambda c: x1_ref[:, _cols(c)], t - 1, True)
    o = attention(fill, [], [None] * 4 + [lambda: ffn2(t - 2, (0, 1))]
                  + [None] * 4 + [lambda: ffn2(t - 2, (2, 3))], 0)
    rest[0]()
    rest[1]()
    x1, h2 = out_proj(t, o)
    rest[2]()
    rest[3]()
    out_copy(t - 1).start()
    t1, t2 = ffn_value_tasks(lambda r: h2[_cols(r)], lambda c: x1[:, _cols(c)], t, False)
    for fl in t1 + t2:
        fl()
    for d in [out_copy(k) for k in range(NTILES - 1)] + last_copies:
        d.wait()


@jax.jit
def pallas_adaLN_cond__sliding_block__dense_activation_silu__prompt_kernel(
        A_x: jax.Array,
        A_wqkv: jax.Array,
        A_wo: jax.Array,
        B_x: jax.Array,
        B_w1: jax.Array,
        B_w2: jax.Array,
        c: jax.Array,
        w_mod: jax.Array,
):
    del B_x
    anyspec = pl.BlockSpec(memory_space=pl.ANY)
    out = pl.pallas_call(
        _kernel,
        in_specs=[anyspec] * 7,
        out_specs=anyspec,
        out_shape=jax.ShapeDtypeStruct((S, D), A_x.dtype),
        scratch_shapes=[
            pltpu.VMEM((S, D), bf16),
            pltpu.VMEM((D, 3 * D), bf16),
            pltpu.VMEM((D, D), bf16),
            pltpu.VMEM((D, F), bf16),
            pltpu.VMEM((F, D), bf16),
            pltpu.VMEM((1, D), bf16),
            pltpu.VMEM((D, 6 * D), bf16),
            pltpu.VMEM((8, 6 * D), f32),
            pltpu.VMEM((D, D), u32),
            pltpu.VMEM((D // 2, TQ), u32),
            pltpu.VMEM((D // 2, TQ), u32),
            pltpu.VMEM((3 * TQ // 2, D), u32),
            pltpu.VMEM((D // 2, 2 * TQ), u32),
            pltpu.VMEM((NCH * 8, NPS * 128), u32),
            pltpu.VMEM((TQ, D), f32),
            pltpu.VMEM((TQ // 2, D), u32),
            pltpu.VMEM((TQ, D), u32),
            pltpu.VMEM((2 * TQ, D), f32),
            pltpu.VMEM((2 * TQ, 2 * D), f32),
            pltpu.VMEM((TQ // 2, F), u32),
            pltpu.VMEM((16, D), f32),
            pltpu.SMEM((1,), jnp.int32),
            pltpu.SemaphoreType.DMA((9,)),
        ],
        compiler_params=pltpu.CompilerParams(vmem_limit_bytes=64 * 1024 * 1024),
    )(A_x.reshape(S, D), A_wqkv, A_wo, B_w1, B_w2, c, w_mod)
    return out.reshape(1, S, D)
```

```python
import functools

import jax
import jax.numpy as jnp
from jax import lax
import jax.experimental.pallas as pl
import jax.experimental.pallas.tpu as pltpu

S, D, DH, F = 2048, 512, 16, 1792
TQ = 256
NTILES = S // TQ
NFC = F // 128
EPS = 1e-5
QSCALE = (DH ** -0.5) * 1.4426950408889634
NEG = -1e30
NCH = 17
NPS = 32
bf16, u32, f32 = jnp.bfloat16, jnp.uint32, jnp.float32
NT_DIMS = (((1,), (1,)), ((), ()))
TILES = [(qb, g, j) for qb in range(TQ // 128) for g in range(4) for j in range(8)]
N = len(TILES)


def _iota(shape, dim):
    return lax.broadcasted_iota(jnp.int32, shape, dim)


def _ln(x):
    xc = x - jnp.mean(x, axis=-1, keepdims=True)
    ss = jnp.sum(xc * xc, axis=-1, keepdims=True) + D * EPS
    return xc * jnp.exp2(-0.5 * jnp.log2(ss))


def _modulate(n, scale, shift):
    return (n * ((1.0 + scale) * D ** 0.5) + shift).astype(bf16)


def _silu(z):
    hz = 0.5 * z
    return hz + hz * jnp.tanh(hz)


def _dot(a, b):
    return jnp.dot(a, b, preferred_element_type=f32)


def _as_bf16(x):
    return pltpu.bitcast(x, bf16)


def _cols(c):
    return slice(c * 128, (c + 1) * 128)


def _slot(n):
    return _cols(n % NPS)


def _col_max(blocks):
    ms = [functools.reduce(lax.max, [b[k:k + 8] for k in range(0, b.shape[0], 8)]) for b in blocks]
    while len(ms) > 1:
        ms = [lax.max(*ms[k:k + 2]) if k + 1 < len(ms) else ms[k] for k in range(0, len(ms), 2)]
    return jnp.max(ms[0], axis=0, keepdims=True)


def _col_sum(p):
    p = p.reshape(-1, 2, 2, 8, 128)
    v = jnp.sum(p[:, :, 0] + p[:, :, 1], axis=0)
    return jnp.sum(v[0] + v[1], axis=0, keepdims=True)


class _Lanes:
    def __init__(self, n):
        self.n, self.w = n, 128 // n
        w = self.w
        self.tri = _iota((w, 128), 0) > (_iota((w, 128), 1) & (w - 1))
        self.bit = {(r, k): (_iota((r, 128), 1) & (w << k)) != 0
                    for r in (1, w // 2, 64) for k in range(n.bit_length() - 1)}
        self.eq = [(_iota((8, 128), 1) & (128 - w)) == a * w for a in range(n)]
        self.zero = {r: jnp.zeros((r, 128), u32) for r in (8, w // 2)}

    def weights(self, q_ref, tile):
        qb, g, j = TILES[tile]
        a = j % self.n
        parts = [self.zero[8]] * 8
        for r in range(self.n):
            hh = g * 8 + j - a + r
            parts[hh % 8] = lax.select(self.eq[(a + r) % self.n],
                                       q_ref[hh * 8:(hh + 1) * 8, _cols(qb)], self.zero[8])
        return _as_bf16(jnp.concatenate(parts, axis=0))

    def unskew(self, xs, outs):
        n = self.n
        rows = next(x for x in xs if x is not None).shape[0]
        memo = {}

        def get(i, k):
            if k == 0:
                return xs[i % n]
            if (i % n, k) not in memo:
                lo, hi = get(i, k - 1), get(i + (1 << (k - 1)), k - 1)
                memo[i % n, k] = None if lo is None and hi is None else lax.select(
                    self.bit[rows, k - 1], self.zero[rows] if hi is None else hi,
                    self.zero[rows] if lo is None else lo)
            return memo[i % n, k]
        return [get(-r, n.bit_length() - 1) for r in outs]


class _Heads:
    def __init__(self, lanes, vt_ref, lazy_from=8):
        self.lanes, self.vt_ref, self.lazy_from = lanes, vt_ref, lazy_from
        self.ls, self.acc, self.ot, self.ob = {}, {}, {}, {}

    def pv(self, n0, outs, pieces, vcol, last):
        _, g, j0 = TILES[n0]
        cols = [self.lanes.unskew(xs, outs) for xs in pieces]
        for q, r in enumerate(outs):
            hh = g * 8 + j0 + r
            o = _dot(_as_bf16(self.vt_ref[hh * 8:(hh + 1) * 8, _cols(vcol)]),
                     _as_bf16(jnp.concatenate([c[q] for c in cols], axis=0)))
            self.acc[n0 + r] = o + self.acc[n0 + r] if n0 + r in self.acc else o
        if last:
            ls = self.lanes.unskew([self.ls[n0 + a] for a in range(self.lanes.n)], outs)
            for r, l in zip(outs, ls):
                k = n0 + r
                self.ot[k] = (self.acc.pop(k) * pl.reciprocal(l, approx=True), self.lanes.w * r)
                if k // 8 < self.lazy_from:
                    self._unrotate(k)
                    if all(kk in self.ot for kk in range(k // 8 * 8, k // 8 * 8 + 8)):
                        self._group(k // 8)

    def _unrotate(self, k):
        o, shift = self.ot[k]
        if shift:
            self.ot[k] = (pltpu.roll(o, 128 - shift, 1), 0)

    def _group(self, gi):
        if gi not in self.ob:
            ks = range(gi * 8, gi * 8 + 8)
            for k in ks:
                self._unrotate(k)
            self.ob[gi] = jnp.concatenate([self.ot[k][0] for k in ks], axis=0).T
        return self.ob[gi]

    def result(self):
        return jnp.concatenate(
            [jnp.concatenate([self._group(qb * 4 + g) for g in range(4)], axis=1)
             for qb in range(TQ // 128)], axis=0)


def _kernel(x_hbm, wqkv_hbm, wo_hbm, w1_hbm, w2_hbm, c_hbm, wmod_hbm, o_hbm,
            x_v, wqkv_v, wo_v, w1_v, w2_v, c_v, wmod_v,
            mod_ref, wqvt_ref, qt_ref, q0_ref, k_ref, vt_ref, p_ref,
            x1_ref, h2_ref, h01_ref, n_ref, acc_ref, a_ref, sc_ref, sems):
    def cp(src, dst, idx, k):
        return pltpu.make_async_copy(src.at[idx], dst.at[idx], sems.at[k])
    al = slice(None)
    mparts = [(0, 256), (256, 384), (384, 512)]
    d_c = cp(c_hbm, c_v, (al, al), 0)
    d_x01 = cp(x_hbm, x_v, (slice(0, 2 * TQ), al), 0)
    d_m = [[cp(wmod_hbm, wmod_v, (al, slice(k * D + a, k * D + b)), (1, 3, 4)[i]) for k in range(2)]
           for i, (a, b) in enumerate(mparts)]
    d_qk = [cp(wqkv_hbm, wqkv_v, (_cols(j), slice(0, 2 * D)), 2 + j) for j in range(4)]
    d_wv = cp(wqkv_hbm, wqkv_v, (al, slice(2 * D, 3 * D)), 5)
    d_wo = cp(wo_hbm, wo_v, (al, al), 6)
    d_mb = cp(wmod_hbm, wmod_v, (al, slice(2 * D, 6 * D)), 6)
    d_x2 = cp(x_hbm, x_v, (slice(2 * TQ, 3 * TQ), al), 6)
    d_w1 = cp(w1_hbm, w1_v, (al, al), 7)
    d_w2 = cp(w2_hbm, w2_v, (al, al), 8)
    d_xr = cp(x_hbm, x_v, (slice(3 * TQ, S), al), 8)
    for d in ([d_c, d_x01] + d_m[0] + [d_qk[0]] + d_m[1] + [d_qk[1]] + d_m[2]
              + [d_qk[2], d_qk[3], d_wv, d_wo, d_mb, d_x2, d_w1, d_w2, d_xr]):
        d.start()

    def rows_of(t):
        return pl.ds(t * TQ if isinstance(t, int) else pl.multiple_of(t * TQ, TQ), TQ)

    def out_copy(t):
        return pltpu.make_async_copy(x_v.at[rows_of(t)], o_hbm.at[rows_of(t)], sems.at[0])

    def modv(k):
        return mod_ref[0:1, k * D:(k + 1) * D]

    def mod_cols(a, b):
        mod_ref[:, a:b] = _dot(sc_ref[...].astype(bf16), wmod_v[:, a:b])[0:8]

    def ln1(t):
        return _modulate(_ln(x_v[rows_of(t), :].astype(f32)), modv(1), modv(0))

    def k_tasks(get_h):
        def run(c):
            k_ref.bitcast(bf16)[2 * TQ:3 * TQ, _cols(c)] = _dot(
                get_h(), wqkv_v[:, _cols(4 + c)]).astype(bf16)
        return [functools.partial(run, c) for c in range(4)]

    def store_q(dst, qt, n):
        rows = []
        for hh in range(D // DH):
            q = qt[hh * DH:(hh + 1) * DH]
            if hh % n:
                q = jnp.concatenate(
                    [pltpu.roll(q[:, _cols(b)], 128 // n * (hh % n), 1) for b in range(2)], axis=1)
            rows.append(q)
        dst.bitcast(bf16)[...] = jnp.concatenate(rows, axis=0).astype(bf16)

    def t_dot(r0, r1, h):
        return lax.dot_general(_as_bf16(wqvt_ref[r0 // 2:r1 // 2, :]), h, NT_DIMS,
                               preferred_element_type=f32)

    def attention_first(fill):
        lanes = _Lanes(4)
        heads = _Heads(lanes, vt_ref, lazy_from=7)
        neg = jnp.full((32, 128), NEG, f32)

        def scores(n):
            qb, g, j = TILES[n]
            ww = lanes.weights(q0_ref, n)
            rows = qb * 128 + 32 * (j % 4 + 1)
            nsp = min(4, rows // 32)
            b = [(rows // 16 * k + nsp - 1) // nsp * 16 for k in range(nsp + 1)]
            s = jnp.concatenate([_dot(_as_bf16(k_ref[b[k] // 2:b[k + 1] // 2, _cols(g)]), ww)
                                 for k in range(nsp)], axis=0)
            last = lax.select(lanes.tri, neg, s[rows - 32:])
            s = jnp.concatenate([s[:rows - 32], last], axis=0) if rows > 32 else last
            p = jnp.exp2(s - _col_max([s[b[k]:b[k + 1]] for k in range(nsp)]))
            p_ref.bitcast(bf16)[0:rows, _slot(n)] = p.astype(bf16)
            heads.ls[n] = _col_sum(p)

        def pv(n0, k):
            qb = TILES[n0][0]
            if k < qb:
                pieces = [[p_ref[0:64, _slot(n0 + a)] for a in range(4)]]
            else:
                pieces = [[p_ref[qb * 64 + t * 16:qb * 64 + (t + 1) * 16, _slot(n0 + a)]
                           if a >= t else None for a in range(4)] for t in range(4)]
            heads.pv(n0, range(4), pieces, k, k == qb)

        due, at = {}, 0
        for n0 in range(0, N, 4):
            qb = TILES[n0][0]
            for k in range(qb + 1):
                at = max(at, n0 + (11, 9)[qb] + 2 * k)
                due.setdefault(at, []).append((n0, k))
        for i in range(at + 1):
            if i < N:
                scores(i - i % 4 + (2, 3, 1, 0)[i % 4])
            if i in fill:
                fill[i]()
            for step in due.get(i, []):
                pv(*step)
        return heads

    def attention(fillers, late, head=(), skip=3):
        lanes = _Lanes(8)
        heads = _Heads(lanes, vt_ref)
        zero_p = jnp.zeros((16, 128), f32)

        def scores(n):
            qb, g, a = TILES[n]
            ww = lanes.weights(qt_ref, n)
            keys = lambda c0, c1: k_ref[(qb * 8 + a + c0) * 8:(qb * 8 + a + c1) * 8, _cols(g)]
            s = [_dot(_as_bf16(keys(c0, c1)), ww) for c0, c1 in ((1, 6), (6, 10), (10, 14))]
            e = _dot(_as_bf16(jnp.concatenate([keys(0, 1), keys(16, 17), keys(14, 16)], axis=0)), ww)
            edge = lax.select(lanes.tri, e[0:16], e[16:32])
            m = _col_max(s + [jnp.concatenate([edge, e[32:]], axis=0)])
            p = jnp.exp2(jnp.concatenate([edge] + s + [e[32:]], axis=0) - m)
            p_ref.bitcast(bf16)[:, _slot(n)] = jnp.concatenate(
                [lax.select(lanes.tri, p[0:16], zero_p), p[16:256],
                 lax.select(lanes.tri, zero_p, p[0:16])], axis=0).astype(bf16)
            heads.ls[n] = _col_sum(p)

        def pv(i):
            n0, k = i // 6 * 8, (1, 0, 2)[i % 3]
            rngs = [(8, 16)] if k == 1 else [(t, t + 1) for t in range(8 * k, 8 * k + 8)]
            pieces = [[p_ref[(t0 - a) * 8:(t1 - a) * 8, _slot(n0 + a)] if 0 <= t0 - a < NCH else None
                       for a in range(8)] for t0, t1 in rngs]
            heads.pv(n0, range(1 - i // 3 % 2, 8, 2), pieces, TILES[n0][0] + k, i % 3 == 2)

        fillers, late, nq = list(fillers), list(late), 0
        for fl in head:
            if fl is None:
                scores(nq)
                nq += 1
            else:
                fl()
        npv, nf = -7 + 3 * nq // 4, -skip
        while npv < 48 or fillers or late:
            for tok in "QFQPQFQPP":
                if tok == "Q" and nq < N:
                    scores(nq)
                    nq += 1
                elif tok == "P":
                    if 0 <= npv < 48:
                        pv(npv)
                    npv += 1
                elif tok == "F":
                    if nf >= 0 and fillers:
                        fillers.pop(0)()
                    elif nq >= N and late:
                        late.pop(0)()
                    nf += 1
        return heads.result()

    def out_proj(t, o, mix=None):
        ys = []
        for r in range(0, TQ, 128):
            ob = o[r:r + 128].astype(bf16)
            if mix is None:
                ys.append(_dot(ob, wo_v[...]))
            else:
                cols = []
                for c in range(4):
                    cols.append(_dot(ob, wo_v[:, _cols(c)]))
                    for fl in mix.pop(0):
                        fl()
                ys.append(jnp.concatenate(cols, axis=1))
        x1 = x_v[rows_of(t), :].astype(f32) + modv(2) * jnp.concatenate(ys, axis=0)
        return x1, _modulate(_ln(x1), modv(4), modv(3))

    def h2_half(r):
        return _as_bf16(h2_ref[r * 64:(r + 1) * 64, :])

    last_copies = []

    def finish(t, c, x1, y):
        out = (x1 + mod_ref[0:1, _cols(20 + c)] * y).astype(bf16)
        if not (isinstance(t, int) and t == NTILES - 1):
            x_v[rows_of(t), _cols(c)] = out
            return
        nr = TQ // 4 if c == 3 else TQ
        for r in range(0, TQ, nr):
            idx = (slice(t * TQ + r, t * TQ + r + nr), _cols(c))
            x_v[idx] = out[r:r + nr]
            last_copies.append(pltpu.make_async_copy(x_v.at[idx], o_hbm.at[idx], sems.at[0]))
            last_copies[-1].start()

    def ffn1_tasks():
        def run(c, r):
            a_ref.bitcast(bf16)[r * 128:(r + 1) * 128, _cols(c)] = _silu(
                _dot(h2_half(r), w1_v[:, _cols(c)])).astype(bf16)
        return [functools.partial(run, c, r) for c in range(NFC) for r in range(2)]

    def ffn2(t, cs):
        for c in cs:
            finish(t, c, x1_ref[:, _cols(c)], _dot(_as_bf16(a_ref[...]), w2_v[:, _cols(c)]))
            x1_ref[:, _cols(c)] = n_ref[0:TQ, _cols(c)]
        if c == 3:
            out_copy(t).start()

    def ffn_value_tasks(get_h2, get_x1, t, split):
        acts, accs = {}, {}

        def run1(c, r):
            acts[(c, r)] = _silu(_dot(get_h2(r), w1_v[:, _cols(c)]))

        def run2(c, k0, k1):
            a = jnp.concatenate(
                [jnp.concatenate([acts[(k, r)] for k in range(k0, k1)], axis=1) for r in range(2)],
                axis=0).astype(bf16)
            y = _dot(a, w2_v[k0 * 128:k1 * 128, _cols(c)])
            if k0 > 0:
                y = y + accs.pop(c)
            if k1 < NFC:
                accs[c] = y
            else:
                finish(t, c, get_x1(c), y)

        t1 = [functools.partial(run1, c, r) for c in range(NFC) for r in range(2)]
        if not split:
            return t1, [functools.partial(run2, c, 0, NFC) for c in range(4)]
        return (t1 + [functools.partial(run2, c, 0, 8) for c in range(4)],
                [functools.partial(run2, c, 8, NFC) for c in range(4)])

    def mid_step(s, get_h, fill, *order):
        o = attention(fill, [lambda: store_q(qt_ref, t_dot(0, D, get_h()) * QSCALE, 8)], *order)
        k_ref[0:TQ // 2, :] = k_ref[TQ // 2:TQ, :]
        k_ref[TQ // 2:TQ, :] = k_ref[TQ:3 * TQ // 2, :]
        x1, h2 = out_proj(s, o)
        h2_ref.bitcast(bf16)[...] = h2
        n_ref[0:TQ, :] = x1
        vt_ref[:, 0:TQ] = vt_ref[:, TQ:2 * TQ]
        vt_ref.bitcast(bf16)[:, TQ:2 * TQ] = t_dot(D, 2 * D, get_h()).astype(bf16)

    d_c.wait()
    d_x01.wait()
    c = c_v[...].astype(f32)
    sc_ref[...] = jnp.broadcast_to(c * jax.nn.sigmoid(c), (16, D))
    n_ref[...] = _ln(x_v[0:2 * TQ, :].astype(f32))
    ha = lambda: _as_bf16(h01_ref[0:TQ // 2, :])
    hb = lambda: _as_bf16(h01_ref[TQ // 2:TQ, :])
    wt = wqvt_ref.bitcast(bf16)

    def h_cols(i):
        a, b = mparts[i]
        mod_cols(a, b)
        mod_cols(D + a, D + b)
        h01_ref.bitcast(bf16)[:, a:b] = _modulate(
            n_ref[:, a:b], mod_ref[0:1, D + a:D + b], mod_ref[0:1, a:b])

    for d in d_m[0]:
        d.wait()
    h_cols(0)
    for j in range(4):
        d_qk[j].wait()
        for d in (d_m[j] if j in (1, 2) else [d_wv] if j == 3 else []):
            d.wait()
        hj = _as_bf16(h01_ref[:, _cols(j)])
        ya = _dot(hj, wqkv_v[_cols(j), 0:D])
        if j in (1, 2):
            h_cols(j)
        y = jnp.concatenate([ya, _dot(hj, wqkv_v[_cols(j), D:2 * D])], axis=1)
        if j > 0:
            y = y + acc_ref[...]
        if j < 3:
            acc_ref[...] = y
        wt[0:D, _cols(j)] = wqkv_v[_cols(j), 0:D].astype(f32).T.astype(bf16)
    store_q(q0_ref, (y[0:TQ, 0:D] * QSCALE).T, 4)
    store_q(qt_ref, (y[TQ:2 * TQ, 0:D] * QSCALE).T, 8)
    k_ref.bitcast(bf16)[0:2 * TQ, :] = y[:, D:2 * D].astype(bf16)
    wt[D:2 * D, :] = wqkv_v[:, 2 * D:3 * D].astype(f32).T.astype(bf16)
    vt_ref.bitcast(bf16)[:, 0:TQ] = t_dot(D, 2 * D, ha()).astype(bf16)

    def v1(r, half):
        vt_ref.bitcast(bf16)[_cols(r), _cols(2 + half)] = t_dot(
            D + r * 128, D + (r + 1) * 128, hb()[_cols(half)]).astype(bf16)
    heads0 = attention_first(dict(zip(
        (3, 11, 12, 18, 40, 64, 66, 68),
        [functools.partial(v1, r, half) for r in range(4) for half in range(2)])))
    d_wo.wait()
    d_mb.wait()
    d_x2.wait()

    def finish_tile0():
        m = [functools.partial(mod_cols, 2 * D + k * 128, 2 * D + (k + 1) * 128) for k in range(16)]
        h01_ref.bitcast(bf16)[0:TQ, :] = ln1(2)
        k = k_tasks(ha)
        x1, h2 = out_proj(0, heads0.result(), [
            m[0:2], m[2:4], m[4:5], [m[5], k[0], m[6], m[7], k[1], m[8], m[9], k[2], m[10], m[11]],
            m[12:13], m[13:14], m[14:15], [m[15], k[3]]])
        x1_ref[...] = x1
        h2_ref.bitcast(bf16)[...] = h2

    def tile1():
        d_w1.wait()
        mid_step(1, ha, ffn1_tasks())

    def two_phases(i, carry):
        pl.when(i == 0)(finish_tile0)
        pl.when(i == 1)(tile1)
        return carry

    lax.fori_loop(0, 2, two_phases, 0)
    d_w2.wait()
    d_xr.wait()

    def body(s, carry):
        h = []

        def finish_old():
            ffn2(s - 2, (0, 1))
            h.append(ln1(s + 1))
            ffn2(s - 2, (2, 3))
        mid_step(s, lambda: h[0], ffn1_tasks() + k_tasks(lambda: h[0]), [None] * 8 + [finish_old], 1)
        return carry

    lax.fori_loop(2, NTILES - 1, body, 0)

    t = NTILES - 1
    fill, rest = ffn_value_tasks(h2_half, lambda c: x1_ref[:, _cols(c)], t - 1, True)
    o = attention(fill, [], [None] * 4 + [lambda: ffn2(t - 2, (0, 1))]
                  + [None] * 4 + [lambda: ffn2(t - 2, (2, 3))], 0)
    rest[0]()
    rest[1]()
    x1, h2 = out_proj(t, o)
    rest[2]()
    rest[3]()
    out_copy(t - 1).start()
    t1, t2 = ffn_value_tasks(lambda r: h2[_cols(r)], lambda c: x1[:, _cols(c)], t, False)
    for fl in t1 + t2:
        fl()
    for d in [out_copy(k) for k in range(NTILES - 1)] + last_copies:
        d.wait()


@jax.jit
def pallas_adaLN_cond__sliding_block__dense_activation_silu__prompt_kernel(
        A_x: jax.Array,
        A_wqkv: jax.Array,
        A_wo: jax.Array,
        B_x: jax.Array,
        B_w1: jax.Array,
        B_w2: jax.Array,
        c: jax.Array,
        w_mod: jax.Array,
):
    del B_x
    anyspec = pl.BlockSpec(memory_space=pl.ANY)
    out = pl.pallas_call(
        _kernel,
        in_specs=[anyspec] * 7,
        out_specs=anyspec,
        out_shape=jax.ShapeDtypeStruct((S, D), A_x.dtype),
        scratch_shapes=[
            pltpu.VMEM((S, D), bf16),
            pltpu.VMEM((D, 3 * D), bf16),
            pltpu.VMEM((D, D), bf16),
            pltpu.VMEM((D, F), bf16),
            pltpu.VMEM((F, D), bf16),
            pltpu.VMEM((1, D), bf16),
            pltpu.VMEM((D, 6 * D), bf16),
            pltpu.VMEM((8, 6 * D), f32),
            pltpu.VMEM((D, D), u32),
            pltpu.VMEM((D // 2, TQ), u32),
            pltpu.VMEM((D // 2, TQ), u32),
            pltpu.VMEM((3 * TQ // 2, D), u32),
            pltpu.VMEM((D // 2, 2 * TQ), u32),
            pltpu.VMEM((NCH * 8, NPS * 128), u32),
            pltpu.VMEM((TQ, D), f32),
            pltpu.VMEM((TQ // 2, D), u32),
            pltpu.VMEM((TQ, D), u32),
            pltpu.VMEM((2 * TQ, D), f32),
            pltpu.VMEM((2 * TQ, 2 * D), f32),
            pltpu.VMEM((TQ // 2, F), u32),
            pltpu.VMEM((16, D), f32),
            pltpu.SemaphoreType.DMA((9,)),
        ],
        compiler_params=pltpu.CompilerParams(vmem_limit_bytes=64 * 1024 * 1024),
    )(A_x.reshape(S, D), A_wqkv, A_wo, B_w1, B_w2, c, w_mod)
    return out.reshape(1, S, D)
```

```python
import functools

import jax
import jax.numpy as jnp
from jax import lax
import jax.experimental.pallas as pl
import jax.experimental.pallas.tpu as pltpu

S, D, DH, F = 2048, 512, 16, 1792
TQ = 256
NTILES = S // TQ
NFC = F // 128
EPS = 1e-5
QSCALE = (DH ** -0.5) * 1.4426950408889634
NEG = -1e30
NCH = 17
NPS = 32
bf16, u32, f32 = jnp.bfloat16, jnp.uint32, jnp.float32
NT_DIMS = (((1,), (1,)), ((), ()))
TILES = [(qb, g, j) for qb in range(TQ // 128) for g in range(4) for j in range(8)]
N = len(TILES)


def _iota(shape, dim):
    return lax.broadcasted_iota(jnp.int32, shape, dim)


def _ln(x):
    xc = x - jnp.mean(x, axis=-1, keepdims=True)
    ss = jnp.sum(xc * xc, axis=-1, keepdims=True) + D * EPS
    return xc * jnp.exp2(-0.5 * jnp.log2(ss))


def _modulate(n, scale, shift):
    return (n * ((1.0 + scale) * D ** 0.5) + shift).astype(bf16)


def _silu(z):
    hz = 0.5 * z
    return hz + hz * jnp.tanh(hz)


def _dot(a, b):
    return jnp.dot(a, b, preferred_element_type=f32)


def _as_bf16(x):
    return pltpu.bitcast(x, bf16)


def _cols(c):
    return slice(c * 128, (c + 1) * 128)


def _slot(n):
    return _cols(n % NPS)


def _col_max(blocks):
    ms = [functools.reduce(lax.max, [b[k:k + 8] for k in range(0, b.shape[0], 8)]) for b in blocks]
    while len(ms) > 1:
        ms = [lax.max(*ms[k:k + 2]) if k + 1 < len(ms) else ms[k] for k in range(0, len(ms), 2)]
    return jnp.max(ms[0], axis=0, keepdims=True)


def _col_sum(p):
    p = p.reshape(-1, 2, 2, 8, 128)
    v = jnp.sum(p[:, :, 0] + p[:, :, 1], axis=0)
    return jnp.sum(v[0] + v[1], axis=0, keepdims=True)


class _Lanes:
    def __init__(self, n):
        self.n, self.w = n, 128 // n
        w = self.w
        self.tri = _iota((w, 128), 0) > (_iota((w, 128), 1) & (w - 1))
        self.bit = {(r, k): (_iota((r, 128), 1) & (w << k)) != 0
                    for r in (1, w // 2, 64) for k in range(n.bit_length() - 1)}
        self.eq = [(_iota((8, 128), 1) & (128 - w)) == a * w for a in range(n)]
        self.zero = {r: jnp.zeros((r, 128), u32) for r in (8, w // 2)}

    def weights(self, q_ref, tile):
        qb, g, j = TILES[tile]
        a = j % self.n
        parts = [self.zero[8]] * 8
        for r in range(self.n):
            hh = g * 8 + j - a + r
            parts[hh % 8] = lax.select(self.eq[(a + r) % self.n],
                                       q_ref[hh * 8:(hh + 1) * 8, _cols(qb)], self.zero[8])
        return _as_bf16(jnp.concatenate(parts, axis=0))

    def unskew(self, xs, outs):
        n = self.n
        rows = next(x for x in xs if x is not None).shape[0]
        memo = {}

        def get(i, k):
            if k == 0:
                return xs[i % n]
            if (i % n, k) not in memo:
                lo, hi = get(i, k - 1), get(i + (1 << (k - 1)), k - 1)
                memo[i % n, k] = None if lo is None and hi is None else lax.select(
                    self.bit[rows, k - 1], self.zero[rows] if hi is None else hi,
                    self.zero[rows] if lo is None else lo)
            return memo[i % n, k]
        return [get(-r, n.bit_length() - 1) for r in outs]


class _Heads:
    def __init__(self, lanes, vt_ref, lazy_from=8):
        self.lanes, self.vt_ref, self.lazy_from = lanes, vt_ref, lazy_from
        self.ls, self.acc, self.ot, self.ob = {}, {}, {}, {}

    def pv(self, n0, outs, pieces, vcol, last):
        _, g, j0 = TILES[n0]
        cols = [self.lanes.unskew(xs, outs) for xs in pieces]
        for q, r in enumerate(outs):
            hh = g * 8 + j0 + r
            o = _dot(_as_bf16(self.vt_ref[hh * 8:(hh + 1) * 8, _cols(vcol)]),
                     _as_bf16(jnp.concatenate([c[q] for c in cols], axis=0)))
            self.acc[n0 + r] = o + self.acc[n0 + r] if n0 + r in self.acc else o
        if last:
            ls = self.lanes.unskew([self.ls[n0 + a] for a in range(self.lanes.n)], outs)
            for r, l in zip(outs, ls):
                k = n0 + r
                self.ot[k] = (self.acc.pop(k) * pl.reciprocal(l, approx=True), self.lanes.w * r)
                if k // 8 < self.lazy_from:
                    self._unrotate(k)
                    if all(kk in self.ot for kk in range(k // 8 * 8, k // 8 * 8 + 8)):
                        self._group(k // 8)

    def _unrotate(self, k):
        o, shift = self.ot[k]
        if shift:
            self.ot[k] = (pltpu.roll(o, 128 - shift, 1), 0)

    def _group(self, gi):
        if gi not in self.ob:
            ks = range(gi * 8, gi * 8 + 8)
            for k in ks:
                self._unrotate(k)
            self.ob[gi] = jnp.concatenate([self.ot[k][0] for k in ks], axis=0).T
        return self.ob[gi]

    def result(self):
        return jnp.concatenate(
            [jnp.concatenate([self._group(qb * 4 + g) for g in range(4)], axis=1)
             for qb in range(TQ // 128)], axis=0)


def _kernel(x_hbm, wqkv_hbm, wo_hbm, w1_hbm, w2_hbm, c_hbm, wmod_hbm, o_hbm,
            x_v, wqkv_v, wo_v, w1_v, w2_v, c_v, wmod_v,
            mod_ref, wqvt_ref, qt_ref, q0_ref, k_ref, vt_ref, p_ref,
            x1_ref, h2_ref, h01_ref, n_ref, acc_ref, a_ref, sc_ref, sems):
    def cp(src, dst, idx, k):
        return pltpu.make_async_copy(src.at[idx], dst.at[idx], sems.at[k])
    al = slice(None)
    mparts = [(0, 256), (256, 384), (384, 512)]
    d_c = cp(c_hbm, c_v, (al, al), 0)
    d_x01 = cp(x_hbm, x_v, (slice(0, 2 * TQ), al), 0)
    d_m = [[cp(wmod_hbm, wmod_v, (al, slice(k * D + a, k * D + b)), (1, 3, 4)[i]) for k in range(2)]
           for i, (a, b) in enumerate(mparts)]
    d_qk = [cp(wqkv_hbm, wqkv_v, (_cols(j), slice(0, 2 * D)), 2 + j) for j in range(4)]
    d_wv = cp(wqkv_hbm, wqkv_v, (al, slice(2 * D, 3 * D)), 5)
    d_wo = cp(wo_hbm, wo_v, (al, al), 6)
    d_mb = cp(wmod_hbm, wmod_v, (al, slice(2 * D, 6 * D)), 6)
    d_x2 = cp(x_hbm, x_v, (slice(2 * TQ, 3 * TQ), al), 6)
    d_w1 = cp(w1_hbm, w1_v, (al, al), 7)
    d_w2 = cp(w2_hbm, w2_v, (al, al), 8)
    d_xr = cp(x_hbm, x_v, (slice(3 * TQ, S), al), 8)
    for d in ([d_c, d_x01] + d_m[0] + [d_qk[0]] + d_m[1] + [d_qk[1]] + d_m[2]
              + [d_qk[2], d_qk[3], d_wv, d_wo, d_mb, d_x2, d_w1, d_w2, d_xr]):
        d.start()

    def rows_of(t):
        return pl.ds(t * TQ if isinstance(t, int) else pl.multiple_of(t * TQ, TQ), TQ)

    def out_copy(t):
        return pltpu.make_async_copy(x_v.at[rows_of(t)], o_hbm.at[rows_of(t)], sems.at[0])

    def modv(k):
        return mod_ref[0:1, k * D:(k + 1) * D]

    def mod_cols(a, b):
        mod_ref[:, a:b] = _dot(sc_ref[...].astype(bf16), wmod_v[:, a:b])[0:8]

    def ln1(t):
        return _modulate(_ln(x_v[rows_of(t), :].astype(f32)), modv(1), modv(0))

    def k_tasks(get_h):
        def run(c):
            k_ref.bitcast(bf16)[2 * TQ:3 * TQ, _cols(c)] = _dot(
                get_h(), wqkv_v[:, _cols(4 + c)]).astype(bf16)
        return [functools.partial(run, c) for c in range(4)]

    def store_q(dst, r0, qt, n):
        rows = []
        for hh in range(qt.shape[0] // DH):
            q = qt[hh * DH:(hh + 1) * DH]
            if hh % n:
                q = jnp.concatenate(
                    [pltpu.roll(q[:, _cols(b)], 128 // n * (hh % n), 1) for b in range(2)], axis=1)
            rows.append(q)
        dst.bitcast(bf16)[r0:r0 + qt.shape[0], :] = jnp.concatenate(rows, axis=0).astype(bf16)

    def t_dot(r0, r1, h):
        return lax.dot_general(_as_bf16(wqvt_ref[r0 // 2:r1 // 2, :]), h, NT_DIMS,
                               preferred_element_type=f32)

    def attention_first(fill):
        lanes = _Lanes(4)
        heads = _Heads(lanes, vt_ref, lazy_from=7)
        neg = jnp.full((32, 128), NEG, f32)

        def scores(n):
            qb, g, j = TILES[n]
            ww = lanes.weights(q0_ref, n)
            rows = qb * 128 + 32 * (j % 4 + 1)
            nsp = min(4, rows // 32)
            b = [(rows // 16 * k + nsp - 1) // nsp * 16 for k in range(nsp + 1)]
            s = jnp.concatenate([_dot(_as_bf16(k_ref[b[k] // 2:b[k + 1] // 2, _cols(g)]), ww)
                                 for k in range(nsp)], axis=0)
            last = lax.select(lanes.tri, neg, s[rows - 32:])
            s = jnp.concatenate([s[:rows - 32], last], axis=0) if rows > 32 else last
            p = jnp.exp2(s - _col_max([s[b[k]:b[k + 1]] for k in range(nsp)]))
            p_ref.bitcast(bf16)[0:rows, _slot(n)] = p.astype(bf16)
            heads.ls[n] = _col_sum(p)

        def pv(n0, k):
            qb = TILES[n0][0]
            if k < qb:
                pieces = [[p_ref[0:64, _slot(n0 + a)] for a in range(4)]]
            else:
                pieces = [[p_ref[qb * 64 + t * 16:qb * 64 + (t + 1) * 16, _slot(n0 + a)]
                           if a >= t else None for a in range(4)] for t in range(4)]
            heads.pv(n0, range(4), pieces, k, k == qb)

        due, at = {}, 0
        for n0 in range(0, N, 4):
            qb = TILES[n0][0]
            for k in range(qb + 1):
                at = max(at, n0 + (11, 9)[qb] + 2 * k)
                due.setdefault(at, []).append((n0, k))
        for i in range(at + 1):
            if i < N:
                scores(i - i % 4 + (2, 3, 1, 0)[i % 4])
            if i in fill:
                fill[i]()
            for step in due.get(i, []):
                pv(*step)
        return heads

    def attention(fillers, late, head=(), skip=3, kord=(1, 0, 2)):
        lanes = _Lanes(8)
        heads = _Heads(lanes, vt_ref)
        zero_p = jnp.zeros((16, 128), f32)

        def scores(n):
            qb, g, a = TILES[n]
            ww = lanes.weights(qt_ref, n)
            keys = lambda c0, c1: k_ref[(qb * 8 + a + c0) * 8:(qb * 8 + a + c1) * 8, _cols(g)]
            s = [_dot(_as_bf16(keys(c0, c1)), ww) for c0, c1 in ((1, 6), (6, 10), (10, 14))]
            e = _dot(_as_bf16(jnp.concatenate([keys(0, 1), keys(16, 17), keys(14, 16)], axis=0)), ww)
            edge = lax.select(lanes.tri, e[0:16], e[16:32])
            m = _col_max(s + [jnp.concatenate([edge, e[32:]], axis=0)])
            p = jnp.exp2(jnp.concatenate([edge] + s + [e[32:]], axis=0) - m)
            p_ref.bitcast(bf16)[:, _slot(n)] = jnp.concatenate(
                [lax.select(lanes.tri, p[0:16], zero_p), p[16:256],
                 lax.select(lanes.tri, zero_p, p[0:16])], axis=0).astype(bf16)
            heads.ls[n] = _col_sum(p)

        def pv(i):
            n0, k = i // 6 * 8, kord[i % 3]
            rngs = [(8, 16)] if k == 1 else [(t, t + 1) for t in range(8 * k, 8 * k + 8)]
            pieces = [[p_ref[(t0 - a) * 8:(t1 - a) * 8, _slot(n0 + a)] if 0 <= t0 - a < NCH else None
                       for a in range(8)] for t0, t1 in rngs]
            heads.pv(n0, range(1 - i // 3 % 2, 8, 2), pieces, TILES[n0][0] + k, i % 3 == 2)

        fillers, late, nq = list(fillers), list(late), 0
        for fl in head:
            if fl is None:
                scores(nq)
                nq += 1
            else:
                fl()
        npv, nf = -7 + 3 * nq // 4, -skip
        while npv < 48 or fillers or late:
            for tok in "QFQPQFQPP":
                if tok == "Q" and nq < N:
                    scores(nq)
                    nq += 1
                elif tok == "P":
                    if 0 <= npv < 48:
                        pv(npv)
                    npv += 1
                elif tok == "F":
                    if nf >= 0 and fillers:
                        fillers.pop(0)()
                    elif nq >= N and late:
                        late.pop(0)()
                    nf += 1
        return heads.result()

    def out_proj(t, o, mix=None):
        ys = []
        for r in range(0, TQ, 128):
            ob = o[r:r + 128].astype(bf16)
            if mix is None:
                ys.append(_dot(ob, wo_v[...]))
            else:
                cols = []
                for c in range(4):
                    cols.append(_dot(ob, wo_v[:, _cols(c)]))
                    for fl in mix.pop(0):
                        fl()
                ys.append(jnp.concatenate(cols, axis=1))
        x1 = x_v[rows_of(t), :].astype(f32) + modv(2) * jnp.concatenate(ys, axis=0)
        return x1, _modulate(_ln(x1), modv(4), modv(3))

    def h2_half(r):
        return _as_bf16(h2_ref[r * 64:(r + 1) * 64, :])

    last_copies = []

    def finish(t, c, x1, y):
        out = (x1 + mod_ref[0:1, _cols(20 + c)] * y).astype(bf16)
        if not (isinstance(t, int) and t == NTILES - 1):
            x_v[rows_of(t), _cols(c)] = out
            return
        nr = TQ // 4 if c == 3 else TQ
        for r in range(0, TQ, nr):
            idx = (slice(t * TQ + r, t * TQ + r + nr), _cols(c))
            x_v[idx] = out[r:r + nr]
            last_copies.append(pltpu.make_async_copy(x_v.at[idx], o_hbm.at[idx], sems.at[0]))
            last_copies[-1].start()

    def ffn1_tasks():
        def run(c, r):
            a_ref.bitcast(bf16)[r * 128:(r + 1) * 128, _cols(c)] = _silu(
                _dot(h2_half(r), w1_v[:, _cols(c)])).astype(bf16)
        return [functools.partial(run, c, r) for c in range(NFC) for r in range(2)]

    def ffn2(t, cs):
        for c in cs:
            finish(t, c, x1_ref[:, _cols(c)], _dot(_as_bf16(a_ref[...]), w2_v[:, _cols(c)]))
            x1_ref[:, _cols(c)] = n_ref[0:TQ, _cols(c)]
        if c == 3:
            out_copy(t).start()

    def ffn_value_tasks(get_h2, get_x1, t, split):
        acts, accs = {}, {}

        def run1(c, r):
            acts[(c, r)] = _silu(_dot(get_h2(r), w1_v[:, _cols(c)]))

        def run2(c, k0, k1):
            a = jnp.concatenate(
                [jnp.concatenate([acts[(k, r)] for k in range(k0, k1)], axis=1) for r in range(2)],
                axis=0).astype(bf16)
            y = _dot(a, w2_v[k0 * 128:k1 * 128, _cols(c)])
            if k0 > 0:
                y = y + accs.pop(c)
            if k1 < NFC:
                accs[c] = y
            else:
                finish(t, c, get_x1(c), y)

        t1 = [functools.partial(run1, c, r) for c in range(NFC) for r in range(2)]
        if not split:
            return t1, [functools.partial(run2, c, 0, NFC) for c in range(4)]
        return (t1 + [functools.partial(run2, c, 0, 8) for c in range(4)],
                [functools.partial(run2, c, 8, NFC) for c in range(4)])

    def mid_step(s, get_h, fill, *order):
        def proj_q(r):
            store_q(qt_ref, r, t_dot(r, r + 128, get_h()) * QSCALE, 8)
        o = attention(fill, [functools.partial(proj_q, r) for r in range(0, D, 128)], *order)
        k_ref[0:TQ // 2, :] = k_ref[TQ // 2:TQ, :]
        k_ref[TQ // 2:TQ, :] = k_ref[TQ:3 * TQ // 2, :]
        x1, h2 = out_proj(s, o)
        h2_ref.bitcast(bf16)[...] = h2
        n_ref[0:TQ, :] = x1
        vt_ref[:, 0:TQ] = vt_ref[:, TQ:2 * TQ]
        vt_ref.bitcast(bf16)[:, TQ:2 * TQ] = t_dot(D, 2 * D, get_h()).astype(bf16)

    d_c.wait()
    d_x01.wait()
    c = c_v[...].astype(f32)
    sc_ref[...] = jnp.broadcast_to(c * jax.nn.sigmoid(c), (16, D))
    n_ref[...] = _ln(x_v[0:2 * TQ, :].astype(f32))
    ha = lambda: _as_bf16(h01_ref[0:TQ // 2, :])
    hb = lambda: _as_bf16(h01_ref[TQ // 2:TQ, :])
    wt = wqvt_ref.bitcast(bf16)

    def h_cols(i):
        a, b = mparts[i]
        mod_cols(a, b)
        mod_cols(D + a, D + b)
        h01_ref.bitcast(bf16)[:, a:b] = _modulate(
            n_ref[:, a:b], mod_ref[0:1, D + a:D + b], mod_ref[0:1, a:b])

    for d in d_m[0]:
        d.wait()
    h_cols(0)
    for j in range(4):
        d_qk[j].wait()
        for d in (d_m[j] if j in (1, 2) else [d_wv] if j == 3 else []):
            d.wait()
        hj = _as_bf16(h01_ref[:, _cols(j)])
        ya = _dot(hj, wqkv_v[_cols(j), 0:D])
        if j in (1, 2):
            h_cols(j)
        y = jnp.concatenate([ya, _dot(hj, wqkv_v[_cols(j), D:2 * D])], axis=1)
        if j > 0:
            y = y + acc_ref[...]
        if j < 3:
            acc_ref[...] = y
        wt[0:D, _cols(j)] = wqkv_v[_cols(j), 0:D].astype(f32).T.astype(bf16)
    store_q(q0_ref, 0, (y[0:TQ, 0:D] * QSCALE).T, 4)
    store_q(qt_ref, 0, (y[TQ:2 * TQ, 0:D] * QSCALE).T, 8)
    k_ref.bitcast(bf16)[0:2 * TQ, :] = y[:, D:2 * D].astype(bf16)
    wt[D:2 * D, :] = wqkv_v[:, 2 * D:3 * D].astype(f32).T.astype(bf16)
    vt_ref.bitcast(bf16)[:, 0:TQ] = t_dot(D, 2 * D, ha()).astype(bf16)

    def v1(r, half):
        vt_ref.bitcast(bf16)[_cols(r), _cols(2 + half)] = t_dot(
            D + r * 128, D + (r + 1) * 128, hb()[_cols(half)]).astype(bf16)
    heads0 = attention_first(dict(zip(
        (3, 11, 12, 18, 40, 64, 66, 68),
        [functools.partial(v1, r, half) for r in range(4) for half in range(2)])))
    d_wo.wait()
    d_mb.wait()
    d_x2.wait()

    def finish_tile0():
        m = [functools.partial(mod_cols, 2 * D + k * 128, 2 * D + (k + 1) * 128) for k in range(16)]
        h01_ref.bitcast(bf16)[0:TQ, :] = ln1(2)
        k = k_tasks(ha)
        x1, h2 = out_proj(0, heads0.result(), [
            m[0:2], m[2:4], m[4:5], [m[5], k[0], m[6], m[7], k[1], m[8], m[9], k[2], m[10], m[11]],
            m[12:13], m[13:14], m[14:15], [m[15], k[3]]])
        x1_ref[...] = x1
        h2_ref.bitcast(bf16)[...] = h2

    def tile1():
        d_w1.wait()
        mid_step(1, ha, ffn1_tasks())

    def two_phases(i, carry):
        pl.when(i == 0)(finish_tile0)
        pl.when(i == 1)(tile1)
        return carry

    lax.fori_loop(0, 2, two_phases, 0)
    d_w2.wait()
    d_xr.wait()

    def body(s, carry):
        h = []

        def finish_old():
            ffn2(s - 2, (0, 1))
            h.append(ln1(s + 1))
            ffn2(s - 2, (2, 3))
        mid_step(s, lambda: h[0], ffn1_tasks() + k_tasks(lambda: h[0]),
                 [None] * 8 + [finish_old], 1, (1, 2, 0))
        return carry

    lax.fori_loop(2, NTILES - 1, body, 0)

    t = NTILES - 1
    fill, rest = ffn_value_tasks(h2_half, lambda c: x1_ref[:, _cols(c)], t - 1, True)
    o = attention(fill, [], [None] * 4 + [lambda: ffn2(t - 2, (0, 1))]
                  + [None] * 4 + [lambda: ffn2(t - 2, (2, 3))], 0)
    rest[0]()
    rest[1]()
    x1, h2 = out_proj(t, o)
    rest[2]()
    rest[3]()
    out_copy(t - 1).start()
    t1, t2 = ffn_value_tasks(lambda r: h2[_cols(r)], lambda c: x1[:, _cols(c)], t, False)
    for fl in t1 + t2:
        fl()
    for d in [out_copy(k) for k in range(NTILES - 1)] + last_copies:
        d.wait()


@jax.jit
def pallas_adaLN_cond__sliding_block__dense_activation_silu__prompt_kernel(
        A_x: jax.Array,
        A_wqkv: jax.Array,
        A_wo: jax.Array,
        B_x: jax.Array,
        B_w1: jax.Array,
        B_w2: jax.Array,
        c: jax.Array,
        w_mod: jax.Array,
):
    del B_x
    anyspec = pl.BlockSpec(memory_space=pl.ANY)
    out = pl.pallas_call(
        _kernel,
        in_specs=[anyspec] * 7,
        out_specs=anyspec,
        out_shape=jax.ShapeDtypeStruct((S, D), A_x.dtype),
        scratch_shapes=[
            pltpu.VMEM((S, D), bf16),
            pltpu.VMEM((D, 3 * D), bf16),
            pltpu.VMEM((D, D), bf16),
            pltpu.VMEM((D, F), bf16),
            pltpu.VMEM((F, D), bf16),
            pltpu.VMEM((1, D), bf16),
            pltpu.VMEM((D, 6 * D), bf16),
            pltpu.VMEM((8, 6 * D), f32),
            pltpu.VMEM((D, D), u32),
            pltpu.VMEM((D // 2, TQ), u32),
            pltpu.VMEM((D // 2, TQ), u32),
            pltpu.VMEM((3 * TQ // 2, D), u32),
            pltpu.VMEM((D // 2, 2 * TQ), u32),
            pltpu.VMEM((NCH * 8, NPS * 128), u32),
            pltpu.VMEM((TQ, D), f32),
            pltpu.VMEM((TQ // 2, D), u32),
            pltpu.VMEM((TQ, D), u32),
            pltpu.VMEM((2 * TQ, D), f32),
            pltpu.VMEM((2 * TQ, 2 * D), f32),
            pltpu.VMEM((TQ // 2, F), u32),
            pltpu.VMEM((16, D), f32),
            pltpu.SemaphoreType.DMA((9,)),
        ],
        compiler_params=pltpu.CompilerParams(vmem_limit_bytes=64 * 1024 * 1024),
    )(A_x.reshape(S, D), A_wqkv, A_wo, B_w1, B_w2, c, w_mod)
    return out.reshape(1, S, D)
```
